```python
import os as _os
_os.environ.setdefault("JAX_PLATFORMS", "cpu")
import jax
import jax.numpy as jnp

def _softmax(x, axis=-1):
    return jax.nn.softmax(x, axis=axis)
def _gelu(x):
    return jax.nn.gelu(x, approximate=True)
def _silu(x):
    return jax.nn.silu(x)
def _sigmoid(x):
    return jax.nn.sigmoid(x)
def _layernorm(x, axis=-1, eps=1e-5):
    m = jnp.mean(x, axis=axis, keepdims=True)
    v = jnp.var(x, axis=axis, keepdims=True)
    return (x - m) / jnp.sqrt(v + eps)
def _scatter_add(tgt, idx, src, axis=0):
    return tgt.at[idx].add(src)
def _segment_sum(src, seg, n):
    return jax.ops.segment_sum(src, seg, n)
class _Rng:
    def __init__(self, key):
        self._k = key
    def _next(self):
        self._k, sub = jax.random.split(self._k)
        return sub
    def normal(self, shape):
        return jax.random.normal(self._next(), shape, dtype=jnp.bfloat16)
    def randint(self, lo, hi, shape):
        return jax.random.randint(self._next(), shape, lo, hi, dtype=jnp.int32)
    def uniform(self, shape, lo=0.0, hi=1.0):
        return jax.random.uniform(self._next(), shape, jnp.bfloat16, lo, hi)
    def permutation(self, n):
        return jax.random.permutation(self._next(), n)


kernel_name = 'parallel_sum__softmax_full_mha__glu_gated_swiglu__prompt'

def setup_inputs():
    _rng = _Rng(jax.random.key(int.from_bytes(__import__("os").urandom(4), "little")))
    _w = (lambda a: (lambda t: t.astype(jnp.bfloat16) if jnp.issubdtype(t.dtype, jnp.floating) else t)(jnp.asarray(a)))
    def _A_setup():
        B, S, D = 1, 2048, 448
        return {
            "x": _w((lambda *s: _rng.normal(s) * 0.05)(B, S, D)),
            "wqkv": _w((lambda *s: _rng.normal(s) * 0.05)(D, 3 * D)),
            "wo": _w((lambda *s: _rng.normal(s) * 0.05)(D, D)),
        }
    _A_in = _A_setup()

    def _B_setup():
        B, S, D, F = 1, 2048, 448, 1792
        return {
            "x": _w((lambda *s: _rng.normal(s) * 0.05)(B, S, D)),
            "w1": _w((lambda *s: _rng.normal(s) * 0.05)(D, F) * (2.0 / D) ** 0.5),
            "w3": _w((lambda *s: _rng.normal(s) * 0.05)(D, F) * (2.0 / D) ** 0.5),
            "w2": _w((lambda *s: _rng.normal(s) * 0.05)(F, D) * (2.0 / F) ** 0.5),
        }
    _B_in = _B_setup()

    return {
        "A_x": _A_in["x"],
        "A_wqkv": _A_in["wqkv"],
        "A_wo": _A_in["wo"],
        "B_x": _B_in["x"],
        "B_w1": _B_in["w1"],
        "B_w3": _B_in["w3"],
        "B_w2": _B_in["w2"],
    }

def reference(A_x, A_wqkv, A_wo, B_x, B_w1, B_w3, B_w2):
    def _A_ref(x, wqkv, wo):
        B, S, D = x.shape
        H = 16; Dh = D // H
        qkv = (lambda x, *d: x.transpose(*d))((x @ wqkv).reshape(B, S, 3, H, Dh), 2, 0, 3, 1, 4)
        q, k, v = qkv[0], qkv[1], qkv[2]
        scale = Dh ** -0.5
        scores = jnp.einsum("bhqd,bhkd->bhqk", q, k) * scale
        p = _softmax(scores, axis=-1)
        o = jnp.einsum("bhqk,bhkd->bhqd", p, v)
        return (lambda x, *d: x.transpose(*d))(o, 0, 2, 1, 3).reshape(B, S, D) @ wo

    def _B_ref(x, w1, w3, w2):
        gate = jnp.einsum("bsd,df->bsf", x, w1)
        up = jnp.einsum("bsd,df->bsf", x, w3)
        h = _silu(gate) * up
        out = jnp.einsum("bsf,fd->bsd", h, w2)
        return out

    x = A_x
    xn = _layernorm(x, axis=-1)
    return x + _A_ref(xn, A_wqkv, A_wo) + _B_ref(xn, B_w1, B_w3, B_w2)
```

```python
import functools
import math

import jax
import jax.numpy as jnp
from jax import lax
import jax.experimental.pallas as pl
import jax.experimental.pallas.tpu as pltpu

H = 16
HP = 32
HPG = 4
LANES = 128
EPS = 1e-5

NT = (((1,), (1,)), ((), ()))
TN = (((0,), (0,)), ((), ()))


def _kernel(x_ref, wqkv_ref, wvt_ref, wo_ref, w1_ref, w3_ref, w2_ref, o_ref,
            xn_sc, q_sc, k_sc, vt_sc, ot_sc, *, S, D, F, TQ, TC, FC):
    Dh = D // H
    G = H // HPG
    GW = HPG * Dh
    qscale = (Dh ** -0.5) * math.log2(math.e)
    i = pl.program_id(0)

    @pl.when(i == 0)
    def _prologue():
        def chunk(c, carry):
            r0 = pl.multiple_of(c * TC, TC)
            x = x_ref[pl.ds(r0, TC), :].astype(jnp.float32)
            mu = jnp.mean(x, axis=-1, keepdims=True)
            xc = x - mu
            var = jnp.mean(xc * xc, axis=-1, keepdims=True)
            xn = (xc * lax.rsqrt(var + EPS)).astype(jnp.bfloat16)
            xn_sc[pl.ds(r0, TC), :] = xn
            for g in range(G):
                wq = wqkv_ref[:, GW * g:GW * g + LANES]
                q = jnp.dot(xn, wq, preferred_element_type=jnp.float32) * qscale
                q_sc[g, pl.ds(r0, TC), :] = q.astype(jnp.bfloat16)
                wk = wqkv_ref[:, D + GW * g:D + GW * g + LANES]
                k = jnp.dot(xn, wk, preferred_element_type=jnp.float32)
                k_sc[g, pl.ds(r0, TC), :] = k.astype(jnp.bfloat16)
            vt = lax.dot_general(wvt_ref[...], xn, NT, preferred_element_type=jnp.float32)
            row = lax.broadcasted_iota(jnp.int32, vt.shape, 0)
            vt = jnp.where(row % HP == Dh, 1.0, vt)
            vt_sc[:, pl.ds(r0, TC)] = vt.astype(jnp.bfloat16)
            return carry
        lax.fori_loop(0, S // TC, chunk, 0)

    q0 = pl.multiple_of(i * TQ, TQ)
    lane = lax.broadcasted_iota(jnp.int32, (TQ, LANES), 1)

    def head(h, carry):
        g = h // HPG
        lo = (h % HPG) * Dh
        qg = q_sc[g, pl.ds(q0, TQ), :]
        qm = jnp.where((lane >= lo) & (lane < lo + Dh), qg, jnp.zeros_like(qg))
        st = lax.dot_general(k_sc[g], qm, NT, preferred_element_type=jnp.float32)
        m = jnp.max(st, axis=0, keepdims=True)
        p = jnp.exp2(st - m).astype(jnp.bfloat16)
        h0 = pl.multiple_of(h * HP, HP)
        ot = jnp.dot(vt_sc[pl.ds(h0, HP), :], p, preferred_element_type=jnp.float32)
        l = ot[Dh:Dh + 1, :]
        ot_sc[pl.ds(h0, HP), :] = ot * (1.0 / l)
        return carry
    lax.fori_loop(0, H, head, 0)

    o = ot_sc[...].T.astype(jnp.bfloat16)
    acc = jnp.dot(o, wo_ref[...], preferred_element_type=jnp.float32)
    acc = acc + x_ref[pl.ds(q0, TQ), :].astype(jnp.float32)
    xn = xn_sc[pl.ds(q0, TQ), :]
    for f in range(F // FC):
        gate = jnp.dot(xn, w1_ref[:, f * FC:(f + 1) * FC], preferred_element_type=jnp.float32)
        up = jnp.dot(xn, w3_ref[:, f * FC:(f + 1) * FC], preferred_element_type=jnp.float32)
        hh = (gate * jax.nn.sigmoid(gate) * up).astype(jnp.bfloat16)
        acc = acc + jnp.dot(hh, w2_ref[f * FC:(f + 1) * FC, :], preferred_element_type=jnp.float32)
    o_ref[...] = acc.astype(o_ref.dtype)


@jax.jit
def pallas_parallel_sum__softmax_full_mha__glu_gated_swiglu__prompt_kernel(
    A_x: jax.Array,
    A_wqkv: jax.Array,
    A_wo: jax.Array,
    B_x: jax.Array,
    B_w1: jax.Array,
    B_w3: jax.Array,
    B_w2: jax.Array,
):
    B, S, D = A_x.shape
    F = B_w1.shape[1]
    Dh = D // H
    TQ = 512
    TC = 512
    FC = 256
    x2 = A_x.reshape(S, D)
    wv = A_wqkv[:, 2 * D:]
    wvt = jnp.pad(wv.reshape(D, H, Dh), ((0, 0), (0, 0), (0, HP - Dh))).reshape(D, H * HP).T
    wo = jnp.pad(A_wo.reshape(H, Dh, D), ((0, 0), (0, HP - Dh), (0, 0))).reshape(H * HP, D)

    full = lambda a: pl.BlockSpec(a.shape, lambda i: (0,) * a.ndim)
    out = pl.pallas_call(
        functools.partial(_kernel, S=S, D=D, F=F, TQ=TQ, TC=TC, FC=FC),
        grid=(S // TQ,),
        in_specs=[full(x2), full(A_wqkv), full(wvt), full(wo), full(B_w1), full(B_w3), full(B_w2)],
        out_specs=pl.BlockSpec((TQ, D), lambda i: (i, 0)),
        out_shape=jax.ShapeDtypeStruct((S, D), A_x.dtype),
        scratch_shapes=[
            pltpu.VMEM((S, D), jnp.bfloat16),
            pltpu.VMEM((H // HPG, S, LANES), jnp.bfloat16),
            pltpu.VMEM((H // HPG, S, LANES), jnp.bfloat16),
            pltpu.VMEM((H * HP, S), jnp.bfloat16),
            pltpu.VMEM((H * HP, TQ), jnp.float32),
        ],
        compiler_params=pltpu.CompilerParams(
            dimension_semantics=("arbitrary",),
            vmem_limit_bytes=100 * 1024 * 1024,
        ),
    )(x2, A_wqkv, wvt, wo, B_w1, B_w3, B_w2)
    return out.reshape(B, S, D)
```

```python
import functools
import math

import jax
import jax.numpy as jnp
from jax import lax
import jax.experimental.pallas as pl
import jax.experimental.pallas.tpu as pltpu

H = 16
HP = 32
HPG = 4
LANES = 128
EPS = 1e-5

NT = (((1,), (1,)), ((), ()))
F32 = jnp.float32
BF16 = jnp.bfloat16

CFG = dict(TQ=512, TC=256, TK=128, GU0=2, SKEW=2, DCH=512, UNR=2, NBUF=4)


def _kernel(xt_hbm, wqkv_hbm, wo_hbm, w1_hbm, w3_hbm, w2t_hbm, o_ref,
            xt_ref, wqkv_ref, wo_ref, w1_ref, w3_ref, w2t_ref, sems,
            xnt_sc, k_sc, vt_sc, wkt_sc, wqt_sc, wvt_sc, wot_sc, h_sc, r_sc, acc_sc, xn_sc, *s_bufs,
            S, D, F, TQ, TC, TK, GU0, SKEW, DCH, UNR, NBUF):
    Dh = D // H
    G = H // HPG
    GW = HPG * Dh
    NC = S // TC
    TF = TQ // G
    NU = F // LANES
    NCH = S // TK
    qscale = (Dh ** -0.5) * math.log2(math.e)
    i = pl.program_id(0)

    def x_copy(c):
        return pltpu.make_async_copy(xt_hbm.at[:, pl.ds(c * TC, TC)],
                                     xt_ref.at[:, pl.ds(c * TC, TC)], sems.at[c])
    w_copies = [pltpu.make_async_copy(src, dst, sems.at[NC + n]) for n, (src, dst) in enumerate(
        [(wo_hbm, wo_ref), (w1_hbm, w1_ref), (w3_hbm, w3_ref), (w2t_hbm, w2t_ref)])]
    wv_copy = pltpu.make_async_copy(wqkv_hbm.at[:, 2 * D:], wqkv_ref.at[:, 2 * D:], sems.at[NC + 4])
    wqk_copy = pltpu.make_async_copy(wqkv_hbm.at[:, :2 * D], wqkv_ref.at[:, :2 * D], sems.at[NC + 5])

    def layernorm(c):
        cols = pl.ds(c * TC, TC)
        x = xt_ref[:, cols].astype(F32)
        mu = jnp.mean(x, axis=0, keepdims=True)
        xc = x - mu
        var = jnp.mean(xc * xc, axis=0, keepdims=True)
        xnt_sc[:, cols] = (xc * lax.rsqrt(var + EPS)).astype(BF16)

    def proj_k(c):
        cols = pl.ds(c * TC, TC)
        kt = jnp.dot(wkt_sc[...], xnt_sc[:, cols], preferred_element_type=F32).astype(BF16)
        for g in range(G):
            k_sc[g, cols, :] = kt[g * GW:(g + 1) * GW, :].T

    def proj_v(c):
        cols = pl.ds(c * TC, TC)
        vt = jnp.dot(wvt_sc[...], xnt_sc[:, cols], preferred_element_type=F32)
        row = lax.broadcasted_iota(jnp.int32, (HP - Dh, TC), 0)
        tail = jnp.where(row == 0, 1.0, 0.0).astype(F32)
        for h in range(H):
            vh = jnp.concatenate([vt[h * Dh:(h + 1) * Dh, :], tail], axis=0)
            vt_sc[h, :, cols] = vh.astype(BF16)

    @pl.when(i == 0)
    def _prologue():
        x_copy(0).start()
        wv_copy.start()
        for c in range(1, NC):
            x_copy(c).start()
        wqk_copy.start()
        for cp in w_copies:
            cp.start()
        r_sc[...] = jnp.zeros(r_sc.shape, F32)
        x_copy(0).wait()
        layernorm(0)
        wv_copy.wait()
        x_copy(1).wait()
        wvt_sc[...] = wqkv_ref[:, 2 * D:].T
        waited = 2
        for c in range(NC):
            if c + 1 < NC and c + 1 >= waited:
                nxt = min(NC, 2 * waited)
                for cc in range(waited, nxt):
                    x_copy(cc).wait()
                waited = nxt
            if c + 1 == NC:
                wqk_copy.wait()
                w_copies[0].wait()
            proj_v(c)
            if c + 1 < NC:
                layernorm(c + 1)
        wqkt = wqkv_ref[:, :2 * D].T
        wkt_sc[...] = wqkt[D:, :]
        for g in range(G):
            wqt_sc[g] = wqkt[g * GW:(g + 1) * GW, :]
        for c in range(NC):
            proj_k(c)
            if c == 1:
                for g in range(G):
                    wot_sc[g] = wo_ref[g * GW:(g + 1) * GW, :].T
        for cp in w_copies[1:]:
            cp.wait()

    q0 = pl.multiple_of(i * TQ, TQ)

    def group(g):
        t0 = pl.multiple_of(q0 + g * TF, TF)
        zoff = pl.multiple_of((g >> 8) * TK, TK)
        xn_sc[0] = xnt_sc[:, pl.ds(t0, TF)].T
        xn = xn_sc[g >> 8]

        def gu_unit(u):
            cols = slice(u * LANES, (u + 1) * LANES)
            gate = jnp.dot(xn, w1_ref[:, cols], preferred_element_type=F32)
            up = jnp.dot(xn, w3_ref[:, cols], preferred_element_type=F32)
            h_sc[:, cols] = (gate * jax.nn.sigmoid(gate) * up).astype(BF16)

        qt = jnp.dot(wqt_sc[g], xnt_sc[:, pl.ds(q0, TQ)], preferred_element_type=F32) * qscale
        row = lax.broadcasted_iota(jnp.int32, (GW, TQ), 0)

        qm = [None] * HPG
        m8 = [None] * HPG
        mx = [None] * HPG
        acc = [None] * HPG

        def a_chunk(j, c):
            if c == 0:
                qm[j] = jnp.where((row >= j * Dh) & (row < (j + 1) * Dh), qt, 0.0).astype(BF16)
            rows = pl.ds(c * TK, TK)
            st = jnp.dot(k_sc[g, rows, :], qm[j], preferred_element_type=F32)
            s_bufs[j % NBUF][rows, :] = st
            cm = jnp.max(st.reshape(TK // 8, 8, TQ), axis=0)
            m8[j] = cm if c == 0 else jnp.maximum(m8[j], cm)
            if c == NCH - 1:
                mx[j] = jnp.max(m8[j], axis=0, keepdims=True)

        def c_chunk(j, c):
            p = jnp.exp2(s_bufs[j % NBUF][pl.ds(zoff + c * TK, TK), :] - mx[j]).astype(BF16)
            pv = jnp.dot(vt_sc[g * HPG + j, :, pl.ds(c * TK, TK)], p, preferred_element_type=F32)
            acc[j] = pv if c == 0 else acc[j] + pv

        for u in range(GU0):
            gu_unit(u)
        NA = HPG * NCH
        lag = NCH + SKEW
        fill = list(range(GU0, NU))
        for n in range(NA + lag):
            if n < NA:
                a_chunk(n // NCH, n % NCH)
            else:
                k = n - NA
                for u in fill[k * len(fill) // lag:(k + 1) * len(fill) // lag]:
                    gu_unit(u)
            if n >= lag:
                c_chunk((n - lag) // NCH, (n - lag) % NCH)
        outs = [a[:Dh, :] * (1.0 / a[Dh:Dh + 1, :]) for a in acc]
        ot = jnp.concatenate(outs, axis=0).astype(BF16)

        r = xt_ref[:, pl.ds(t0, TF)].astype(F32)
        for f0 in range(0, F, DCH):
            f1 = min(f0 + DCH, F)
            r = r + lax.dot_general(w2t_ref[:, f0:f1], h_sc[:, f0:f1], NT, preferred_element_type=F32)
        r_sc[g] = r
        at = jnp.dot(wot_sc[g], ot, preferred_element_type=F32)
        at = at + jnp.where(g == 0, 0.0, acc_sc[...])
        acc_sc[...] = at
        return at

    def body(it, carry):
        for u in range(UNR):
            at = group(it * UNR + u)
        for t in range(G):
            o_ref[:, t * TF:(t + 1) * TF] = (at[:, t * TF:(t + 1) * TF] + r_sc[t]).astype(o_ref.dtype)
        return carry

    lax.fori_loop(0, G // UNR, body, 0)


@jax.jit
def pallas_parallel_sum__softmax_full_mha__glu_gated_swiglu__prompt_kernel(
    A_x: jax.Array,
    A_wqkv: jax.Array,
    A_wo: jax.Array,
    B_x: jax.Array,
    B_w1: jax.Array,
    B_w3: jax.Array,
    B_w2: jax.Array,
):
    B, S, D = A_x.shape
    F = B_w1.shape[1]
    TQ, TC = CFG["TQ"], CFG["TC"]
    G = H // HPG
    GW = HPG * (D // H)
    xt = A_x.reshape(S, D).T
    w2t = B_w2.T

    ins = (xt, A_wqkv, A_wo, B_w1, B_w3, w2t)
    out = pl.pallas_call(
        functools.partial(_kernel, S=S, D=D, F=F, **CFG),
        grid=(S // TQ,),
        in_specs=[pl.BlockSpec(memory_space=pl.ANY)] * len(ins),
        out_specs=pl.BlockSpec((D, TQ), lambda i: (0, i)),
        out_shape=jax.ShapeDtypeStruct((D, S), A_x.dtype),
        scratch_shapes=[pltpu.VMEM(a.shape, a.dtype) for a in ins] + [
            pltpu.SemaphoreType.DMA((S // TC + 6,)),
            pltpu.VMEM((D, S), BF16),
            pltpu.VMEM((G, S, GW), BF16),
            pltpu.VMEM((H, HP, S), BF16),
            pltpu.VMEM((D, D), BF16),
            pltpu.VMEM((G, GW, D), BF16),
            pltpu.VMEM((D, D), BF16),
            pltpu.VMEM((G, D, GW), BF16),
            pltpu.VMEM((TQ // G, F), BF16),
            pltpu.VMEM((G, D, TQ // G), F32),
            pltpu.VMEM((D, TQ), F32),
            pltpu.VMEM((2, TQ // G, D), BF16),
        ] + [pltpu.VMEM((S, TQ), F32)] * CFG["NBUF"],
        compiler_params=pltpu.CompilerParams(
            dimension_semantics=("arbitrary",),
            vmem_limit_bytes=100 * 1024 * 1024,
        ),
    )(*ins)
    return out.T.reshape(B, S, D)
```

```python
import functools
import math

import jax
import jax.numpy as jnp
from jax import lax
import jax.experimental.pallas as pl
import jax.experimental.pallas.tpu as pltpu

H = 16
HP = 32
HPG = 4
LANES = 128
EPS = 1e-5
KPAD = 64

NT = (((1,), (1,)), ((), ()))
F32 = jnp.float32
BF16 = jnp.bfloat16

CFG = dict(TQ=512, TC=256, TK=128, GU0=7, SKEW=18, DCH=512, VC=2200, VR=2, DS=2, ROT=3,
           WG=70, GATE=3, RA=160, SK2=3, PG=3, DFULL=0, DSP=4, SCOPE=0)


def _vchunks(vc):
    return [int(ch) for ch in str(vc).zfill(HPG)]


def _kernel(xt_hbm, wqkv_hbm, wo_hbm, w1_hbm, w3_hbm, w2t_hbm, o_ref,
            xt_ref, wqkv_ref, wo_ref, w1_ref, w3_ref, w2t_ref, sems,
            xnt_sc, k_sc, vt_sc, wkt_sc, wqt_sc, wvt_sc, wot_sc, h_sc, acc_sc, xn_sc, kb_sc, qb_sc, m_sc,
            *s_bufs, S, D, F, TQ, TC, TK, GU0, SKEW, DCH, VC, VR, DS, ROT, WG, GATE, RA, SK2, PG,
            DFULL, DSP, SCOPE):
    Dh = D // H
    G = H // HPG
    GW = HPG * Dh
    NC = S // TC
    NQ = S // TQ
    TF = TQ // G
    NU = F // LANES
    NCH = S // TK
    NQT = TQ // LANES
    BR = 8 * VR
    qscale = (Dh ** -0.5) * math.log2(math.e)
    vch = _vchunks(VC)
    NBC = TK // BR
    vblocks = [(j, b) for j in range(HPG) for b in range(vch[j] * NBC)]
    BLK = Dh
    KBG = len(vblocks) * BLK
    CH = 2 * KBG
    g = pl.program_id(0)
    i = pl.program_id(1)
    zrow = i >> 8

    def x_copy(c):
        return pltpu.make_async_copy(xt_hbm.at[:, pl.ds(c * TC, TC)],
                                     xt_ref.at[:, pl.ds(c * TC, TC)], sems.at[c])
    w_copies = [pltpu.make_async_copy(src, dst, sems.at[NC + n]) for n, (src, dst) in enumerate(
        [(wo_hbm, wo_ref), (w1_hbm, w1_ref), (w3_hbm, w3_ref), (w2t_hbm, w2t_ref)])]
    wv_copy = pltpu.make_async_copy(wqkv_hbm.at[:, 2 * D:], wqkv_ref.at[:, 2 * D:], sems.at[NC + 4])
    wqk_copy = pltpu.make_async_copy(wqkv_hbm.at[:, :2 * D], wqkv_ref.at[:, :2 * D], sems.at[NC + 5])

    def layernorm(c):
        cols = pl.ds(c * TC, TC)
        x = xt_ref[:, cols].astype(F32)
        mu = jnp.mean(x, axis=0, keepdims=True)
        xc = x - mu
        var = jnp.mean(xc * xc, axis=0, keepdims=True)
        xnt_sc[:, cols] = (xc * lax.rsqrt(var + EPS)).astype(BF16)

    def proj_k(c):
        cols = pl.ds(c * TC, TC)
        kt = jnp.dot(wkt_sc[...], xnt_sc[:, cols], preferred_element_type=F32).astype(BF16)
        for gg in range(G):
            k_sc[gg, cols, :] = kt[gg * GW:(gg + 1) * GW, :].T

    def proj_v(c):
        cols = pl.ds(c * TC, TC)
        rc = pl.ds(pl.multiple_of(zrow * TC + c * TC, TC), TC)
        vt = jnp.dot(wvt_sc[...], xnt_sc[:, rc], preferred_element_type=F32)
        row = lax.broadcasted_iota(jnp.int32, (HP - Dh, TC), 0)
        tail = jnp.where(row == 0, 1.0, 0.0).astype(F32)
        for h in range(H):
            vh = jnp.concatenate([vt[h * Dh:(h + 1) * Dh, :], tail], axis=0)
            vt_sc[h, :, cols] = vh.astype(BF16)

    def make_kb(gg, slot, part):
        n0 = 0
        for j in range(HPG):
            nb = vch[j] * NBC // NQ
            if nb:
                r0 = part * (nb * BR)
                base = slot * KBG + (n0 + part * nb) * BLK
                if not isinstance(part, int):
                    r0 = pl.multiple_of(r0, nb * BR)
                kf = k_sc[gg, pl.ds(r0, nb * BR), :].astype(F32)
                for d in range(Dh):
                    kb = jnp.broadcast_to(kf[:, j * Dh + d:j * Dh + d + 1], (nb * BR, LANES))
                    for b in range(nb):
                        kb_sc[base + b * BLK + d] = kb[b * BR:(b + 1) * BR, :]
            n0 += vch[j] * NBC

    def _prologue():
        wv_copy.start()
        for c in range(NC):
            x_copy(c).start()
        wqk_copy.start()
        for cp in w_copies:
            cp.start()
        wv_copy.wait()
        wvt_sc[...] = wqkv_ref[:, 2 * D:].T
        x_copy(0).wait()
        layernorm(0)
        x_copy(1).wait()
        waited = 2
        for c in range(NC - 1):
            if c + 1 >= waited:
                nxt = min(NC, 2 * waited)
                for cc in range(waited, nxt):
                    x_copy(cc).wait()
                waited = nxt
            if c + 2 == NC:
                wqk_copy.wait()
                w_copies[0].wait()
            proj_v(c)
            if c + 2 < NC:
                layernorm(c + 1)
            if c + 3 == NC:
                layernorm(c + 2)
        wqkt = wqkv_ref[:, :2 * D].T
        wkt_sc[...] = wqkt[D:, :]
        for gg in range(G):
            wqt_sc[gg] = wqkt[gg * GW:(gg + 1) * GW, :]
        kb_first = -(-max(vch) * TK // TC)
        for c in range(NC):
            proj_k(c)
            if c == 1:
                for gg in range(G):
                    wot_sc[gg] = wo_ref[gg * GW:(gg + 1) * GW, :].T
            if vblocks and kb_first <= c < kb_first + NQ:
                make_kb(0, 0, c - kb_first)
        proj_v(NC - 1)
        for cp in w_copies[1:]:
            cp.wait()

    def _body():
        q0 = pl.multiple_of(i * TQ, TQ)
        zoff = pl.multiple_of(zrow * TK, TK)
        t0 = pl.multiple_of(q0 + g * TF, TF)
        xn_sc[0] = xnt_sc[:, pl.ds(t0, TF)].T
        xn = xn_sc[zrow]

        qt = jnp.dot(wqt_sc[g], xnt_sc[:, pl.ds(q0, TQ)], preferred_element_type=F32) * qscale
        row = lax.broadcasted_iota(jnp.int32, (GW, TQ), 0)
        qb_sc[0] = qt

        qm = [None] * HPG
        m8 = [None] * HPG
        m8v = [None] * HPG
        mx = [None] * HPG
        acc = [None] * HPG
        outs = [None] * HPG
        kbase = (g % 2) * KBG + zrow
        nah = [NCH - vch[j] for j in range(HPG)]
        left = [nah[j] + vch[j] * NBC for j in range(HPG)]
        lefta = list(nah)
        chain, fin, toks, rot = [], [], [], [0]
        vacc, gates, dacc = {}, {}, {}

        def fold_max(j, cm, mm):
            mm[j] = cm if mm[j] is None else jnp.maximum(mm[j], cm)
            left[j] -= 1
            if mm is m8:
                lefta[j] -= 1
                if lefta[j] == 0 and vch[j]:
                    m_sc[j] = m8[j]
            if left[j] == 0:
                full = m8[j] if m8v[j] is None else jnp.maximum(m_sc[zrow + j], m8v[j])
                mx[j] = jnp.max(full, axis=0, keepdims=True)

        def v_step(n, d):
            j, b = vblocks[n]
            accs = vacc.setdefault(n, [None] * NQT)
            ln = j * Dh + d
            kb = kb_sc[kbase + n * Dh + d]
            for t in range(NQT):
                pr = kb * qb_sc[zrow, ln:ln + 1, t * LANES:(t + 1) * LANES]
                accs[t] = pr if accs[t] is None else accs[t] + pr
            if (d + 1) % DS == 0:
                rot[0] = (rot[0] + ROT) % (VR * NQT)
                v = rot[0] % VR
                chain.append(accs[rot[0] // VR][8 * v:8 * v + 8, :])
                if len(chain) > 1:
                    kb_sc[CH, 0:8, :] = chain.pop(0)
                if fin:
                    kb_sc[CH, 8:16, :] = fin.pop(0)
            if d == Dh - 1:
                st = jnp.concatenate(accs, axis=1)
                s_bufs[j][b * BR:(b + 1) * BR, :] = st
                fold_max(j, jnp.max(st.reshape(VR, 8, TQ), axis=0), m8v)
                fin.extend(m8v[j][:, t * LANES:(t + 1) * LANES] for t in range(NQT))

        def a_chunk(j, c):
            if qm[j] is None:
                qm[j] = jnp.where((row >= j * Dh) & (row < (j + 1) * Dh), qt, 0.0).astype(BF16)
            rows = pl.ds(c * TK, TK)
            st = jnp.dot(k_sc[g, rows, :], qm[j], preferred_element_type=F32)
            s_bufs[j][rows, :] = st
            fold_max(j, jnp.max(st.reshape(TK // 8, 8, TQ), axis=0), m8)
            toks.append(st[TK - 8:, :])

        def c_chunk(j, c):
            if j == 0 and c == 0 and vblocks:
                s_bufs[0][S:S + 8, :] = toks[-GATE]
                s_bufs[0][S:S + 8, :] = m8v[vblocks[-1][0]]
            p = jnp.exp2(s_bufs[j][pl.ds(zoff + c * TK, TK), :] - mx[j]).astype(BF16)
            pv = jnp.dot(vt_sc[g * HPG + j, :, pl.ds(c * TK, TK)], p, preferred_element_type=F32)
            acc[j] = pv if c == 0 else acc[j] + pv
            if c == NCH - 1:
                outs[j] = acc[j][:Dh, :] * (1.0 / acc[j][Dh:Dh + 1, :])

        def gate_task(u):
            gates[u] = jnp.dot(xn, w1_ref[:, u * LANES:(u + 1) * LANES], preferred_element_type=F32)

        def up_task(u):
            hg = 0.5 * gates.pop(u)
            up = jnp.dot(xn, w3_ref[:, u * LANES:(u + 1) * LANES], preferred_element_type=F32)
            h_sc[:, u * LANES:(u + 1) * LANES] = ((hg + hg * jnp.tanh(hg)) * up).astype(BF16)

        MS = D // DSP

        def down_task(f, m):
            part = lax.dot_general(w2t_ref[m * MS:(m + 1) * MS, f * DCH:(f + 1) * DCH],
                                   h_sc[:, f * DCH:(f + 1) * DCH], NT, preferred_element_type=F32)
            dacc[m] = part if m not in dacc else dacc[m] + part

        main = []
        for u in range(GU0):
            main += [(functools.partial(gate_task, u), WG), (functools.partial(up_task, u), WG)]
        a0 = len(main)
        a_list = [(j, c) for j in range(HPG) for c in range(vch[j], NCH)]
        NA = len(a_list)
        for n, (j, c) in enumerate(a_list):
            main.append((functools.partial(a_chunk, j, c), 100 if n <= nah[0] + SKEW - GATE else 0))
        for u in range(GU0, NU):
            main += [(functools.partial(gate_task, u), 0), (functools.partial(up_task, u), 0)]
        for m in range(DSP):
            main += [(functools.partial(down_task, f, m), 0) for f in range(DFULL)]
        riders = [[] for _ in main]
        c_list = [(j, c) for j in range(HPG) for c in range(NCH)]
        nxt, credit = 0, 0
        for slot in range(nah[0] + SKEW, NA):
            credit += RA
            while credit >= 100 and nxt < len(c_list) and slot >= sum(nah[:c_list[nxt][0] + 1]) + SK2:
                riders[a0 + slot].append(functools.partial(c_chunk, *c_list[nxt]))
                nxt += 1
                credit -= 100
            credit = min(credit, 100)
        late = [functools.partial(c_chunk, *jc) for jc in c_list[nxt:]]
        post = list(range(a0 + NA, len(main)))
        for n, rd in enumerate(late):
            riders[post[((n + 1) * len(post) - 1) // len(late)]].append(rd)
        vsteps = [(n, d) for n in range(len(vblocks)) for d in range(Dh)]
        NVS = len(vsteps)
        wtot = sum(w for _, w in main)
        cum, done = 0, 0
        for k, (fn, w) in enumerate(main):
            cum += w
            while done < NVS and done * wtot < cum * NVS:
                v_step(*vsteps[done])
                done += 1
            fn()
            for rd in riders[k]:
                rd()
        ot = jnp.concatenate(outs, axis=0).astype(BF16)
        if vblocks:
            k_sc[0, S:S + 16, :] = outs[PG][0:16, 0:GW].astype(BF16)
            make_kb((g + 1) % G, (g + 1) % 2, i)

        r = xt_ref[:, pl.ds(t0, TF)].astype(F32)
        if DFULL:
            r = r + jnp.concatenate([dacc[m] for m in range(DSP)], axis=0)
        for f0 in range(DFULL * DCH, F, DCH):
            f1 = min(f0 + DCH, F)
            r = r + lax.dot_general(w2t_ref[:, f0:f1], h_sc[:, f0:f1], NT, preferred_element_type=F32)
        at = jnp.dot(wot_sc[g], ot, preferred_element_type=F32)
        for t in range(G):
            cols = slice(t * TF, (t + 1) * TF)
            prev = jnp.where(g == 0, 0.0, acc_sc[i, :, cols]) + jnp.where(g == t, r, 0.0)
            a_t = at[:, cols] + prev
            acc_sc[i, :, cols] = a_t
            o_ref[:, cols] = a_t.astype(o_ref.dtype)

    first = jnp.logical_and(g == 0, i == 0)
    if SCOPE:
        with jax.named_scope("prologue"):
            pl.when(first)(_prologue)
        with jax.named_scope("body"):
            _body()
    else:
        pl.when(first)(_prologue)
        _body()


@jax.jit
def pallas_parallel_sum__softmax_full_mha__glu_gated_swiglu__prompt_kernel(
    A_x: jax.Array,
    A_wqkv: jax.Array,
    A_wo: jax.Array,
    B_x: jax.Array,
    B_w1: jax.Array,
    B_w3: jax.Array,
    B_w2: jax.Array,
):
    B, S, D = A_x.shape
    F = B_w1.shape[1]
    TQ, TC = CFG["TQ"], CFG["TC"]
    G = H // HPG
    Dh = D // H
    GW = HPG * Dh
    BR = 8 * CFG["VR"]
    nkb = 2 * sum(_vchunks(CFG["VC"])) * (CFG["TK"] // BR) * Dh
    xt = A_x.reshape(S, D).T
    w2t = B_w2.T

    ins = (xt, A_wqkv, A_wo, B_w1, B_w3, w2t)
    out = pl.pallas_call(
        functools.partial(_kernel, S=S, D=D, F=F, **CFG),
        grid=(G, S // TQ),
        in_specs=[pl.BlockSpec(memory_space=pl.ANY)] * len(ins),
        out_specs=pl.BlockSpec((D, TQ), lambda g, i: (0, jnp.where(g == G - 1, i, 0))),
        out_shape=jax.ShapeDtypeStruct((D, S), A_x.dtype),
        scratch_shapes=[pltpu.VMEM(a.shape, a.dtype) for a in ins] + [
            pltpu.SemaphoreType.DMA((S // TC + 6,)),
            pltpu.VMEM((D, S), BF16),
            pltpu.VMEM((G, S + KPAD, GW), BF16),
            pltpu.VMEM((H, HP, S), BF16),
            pltpu.VMEM((D, D), BF16),
            pltpu.VMEM((G, GW, D), BF16),
            pltpu.VMEM((D, D), BF16),
            pltpu.VMEM((G, D, GW), BF16),
            pltpu.VMEM((TQ // G, F), BF16),
            pltpu.VMEM((S // TQ, D, TQ), F32),
            pltpu.VMEM((2, TQ // G, D), BF16),
            pltpu.VMEM((nkb + 2, BR, LANES), F32),
            pltpu.VMEM((2, GW, TQ), F32),
            pltpu.VMEM((HPG, 8, TQ), F32),
        ] + [pltpu.VMEM((S + 8, TQ), F32)] * HPG,
        compiler_params=pltpu.CompilerParams(
            dimension_semantics=("arbitrary", "arbitrary"),
            vmem_limit_bytes=110 * 1024 * 1024,
        ),
    )(*ins)
    return out.T.reshape(B, S, D)
```

```python
import functools
import math

import jax
import jax.numpy as jnp
from jax import lax
import jax.experimental.pallas as pl
import jax.experimental.pallas.tpu as pltpu

H = 16
HP = 32
HPG = 4
LANES = 128
EPS = 1e-5
KPAD = 64
VU = 64

NT = (((1,), (1,)), ((), ()))
F32 = jnp.float32
BF16 = jnp.bfloat16

CFG = dict(TQ=512, TC=256, TK=128, GU0=9, WIN=4992, VC=4440, DW=0, WD=100, VR=2, DS=3, LAG=1, ROT=3,
           WG=70, GATE=3, PA=48, SK2=384, PGU=64, LSK=2, PG=63, PN=1, SCOPE=0)


def _vchunks(vc):
    return [int(ch) for ch in str(vc).zfill(HPG)]


def _kernel(xt_hbm, wqkv_hbm, wo_hbm, w1_hbm, w3_hbm, w2t_hbm, o_ref,
            xt_ref, wqkv_ref, wo_ref, w1_ref, w3_ref, w2t_ref, sems,
            xnt_sc, k_sc, vt_sc, wkt_sc, wqt_sc, wvt_sc, wot_sc, h_sc, acc_sc, xn_sc, kb_sc, qb_sc, m_sc, kf_sc, r_sc,
            *s_bufs, S, D, F, TQ, TC, TK, GU0, WIN, VC, DW, WD, VR, DS, LAG, ROT, WG, GATE, PA, SK2, PGU, LSK, PG, PN,
            SCOPE):
    Dh = D // H
    G = H // HPG
    GW = HPG * Dh
    NC = S // TC
    NQ = S // TQ
    TF = TQ // G
    NU = F // LANES
    NCH = S // TK
    NQT = TQ // LANES
    BR = 8 * VR
    qscale = (Dh ** -0.5) * math.log2(math.e)
    vch = _vchunks(VC)
    NBC = VU // BR
    NVR = max(vch) * VU
    vblocks = [(j, b) for j in range(HPG) for b in range(vch[j] * NBC)]
    BLK = Dh
    KBG = len(vblocks) * BLK
    CH = 2 * KBG
    g = pl.program_id(0)
    i = pl.program_id(1)
    zrow = i >> 8

    def x_copy(c):
        return pltpu.make_async_copy(xt_hbm.at[:, pl.ds(c * TC, TC)],
                                     xt_ref.at[:, pl.ds(c * TC, TC)], sems.at[c])
    w_copies = [pltpu.make_async_copy(src, dst, sems.at[NC + n]) for n, (src, dst) in enumerate(
        [(wo_hbm, wo_ref), (w1_hbm, w1_ref), (w3_hbm, w3_ref), (w2t_hbm, w2t_ref)])]
    wv_copy = pltpu.make_async_copy(wqkv_hbm.at[:, 2 * D:], wqkv_ref.at[:, 2 * D:], sems.at[NC + 4])
    wqk_copy = pltpu.make_async_copy(wqkv_hbm.at[:, :2 * D], wqkv_ref.at[:, :2 * D], sems.at[NC + 5])

    def layernorm(c):
        cols = pl.ds(c * TC, TC)
        x = xt_ref[:, cols].astype(F32)
        mu = jnp.mean(x, axis=0, keepdims=True)
        xc = x - mu
        var = jnp.mean(xc * xc, axis=0, keepdims=True)
        xnt_sc[:, cols] = (xc * lax.rsqrt(var + EPS)).astype(BF16)

    def proj_k(c):
        cols = pl.ds(c * TC, TC)
        kt = jnp.dot(wkt_sc[...], xnt_sc[:, cols], preferred_element_type=F32).astype(BF16)
        for gg in range(G):
            kg = kt[gg * GW:(gg + 1) * GW, :].T
            k_sc[gg, cols, :] = kg
            if c * TC < NVR:
                nr = min(TC, NVR - c * TC)
                kf_sc[gg, c * TC:c * TC + nr, :] = kg[:nr, :]

    def proj_v(c):
        cols = pl.ds(c * TC, TC)
        rc = pl.ds(pl.multiple_of(zrow * TC + c * TC, TC), TC)
        vt = jnp.dot(wvt_sc[...], xnt_sc[:, rc], preferred_element_type=F32)
        row = lax.broadcasted_iota(jnp.int32, (HP - Dh, TC), 0)
        tail = jnp.where(row == 0, 1.0, 0.0).astype(F32)
        for h in range(H):
            vh = jnp.concatenate([vt[h * Dh:(h + 1) * Dh, :], tail], axis=0)
            vt_sc[h, :, cols] = vh.astype(BF16)

    kb_items = [(j, d) for j in range(HPG) if vch[j] for d in range(Dh)]

    def make_kb(gg, slot, part, items):
        kf = {}
        for j, d in items:
            nb = vch[j] * NBC // NQ
            base = slot * KBG + (sum(vch[:j]) * NBC + part * nb) * BLK
            if nb not in kf:
                r0 = part * (nb * BR)
                if not isinstance(part, int):
                    r0 = pl.multiple_of(r0, nb * BR)
                kf[nb] = kf_sc[gg, pl.ds(r0, nb * BR), :].astype(F32)
            kb = jnp.broadcast_to(kf[nb][:, j * Dh + d:j * Dh + d + 1], (nb * BR, LANES))
            for b in range(nb):
                kb_sc[base + b * BLK + d] = kb[b * BR:(b + 1) * BR, :]

    def _prologue():
        wv_copy.start()
        for c in range(NC):
            x_copy(c).start()
        wqk_copy.start()
        for cp in w_copies:
            cp.start()
        wv_copy.wait()
        wvt_sc[...] = wqkv_ref[:, 2 * D:].T
        x_copy(0).wait()
        layernorm(0)
        x_copy(1).wait()
        waited = 2
        for c in range(NC - 1):
            if c + 1 >= waited:
                nxt = min(NC, 2 * waited)
                for cc in range(waited, nxt):
                    x_copy(cc).wait()
                waited = nxt
            if c + 2 == NC:
                wqk_copy.wait()
                w_copies[0].wait()
            proj_v(c)
            if c + 2 < NC:
                layernorm(c + 1)
            if c + 3 == NC:
                layernorm(c + 2)
        wqkt = wqkv_ref[:, :2 * D].T
        wkt_sc[...] = wqkt[D:, :]
        for gg in range(G):
            wqt_sc[gg] = wqkt[gg * GW:(gg + 1) * GW, :]
        kb_first = -(-NVR // TC)
        for c in range(NC):
            proj_k(c)
            if c == 1:
                for gg in range(G):
                    wot_sc[gg] = wo_ref[gg * GW:(gg + 1) * GW, :].T
            if vblocks and kb_first <= c < kb_first + NQ:
                make_kb(0, 0, c - kb_first, kb_items)
        proj_v(NC - 1)
        for cp in w_copies[1:]:
            cp.wait()

    def _body():
        q0 = pl.multiple_of(i * TQ, TQ)
        zoff = pl.multiple_of(zrow * TK, TK)
        t0 = pl.multiple_of(q0 + g * TF, TF)
        xn_sc[0] = xnt_sc[:, pl.ds(t0, TF)].T
        xn = xn_sc[zrow]

        qt = jnp.dot(wqt_sc[g], xnt_sc[:, pl.ds(q0, TQ)], preferred_element_type=F32) * qscale
        row = lax.broadcasted_iota(jnp.int32, (GW, TQ), 0)
        qb_sc[0] = qt

        qm = [None] * HPG
        m8 = [None] * HPG
        m8v = [None] * HPG
        mx = [None] * HPG
        acc = [None] * HPG
        outs = [None] * HPG
        kbase = (g % 2) * KBG + zrow
        left = [S] * HPG
        lefta = [S - vch[j] * VU for j in range(HPG)]
        chain, fin, toks, rot = [], [], [], [0]
        vacc, gates = {}, {}

        def fold_max(j, cm, mm, nrows):
            mm[j] = cm if mm[j] is None else jnp.maximum(mm[j], cm)
            left[j] -= nrows
            if mm is m8:
                lefta[j] -= nrows
                if lefta[j] == 0 and vch[j]:
                    m_sc[j] = m8[j]
            if left[j] == 0:
                full = m8[j] if m8v[j] is None else jnp.maximum(m_sc[zrow + j], m8v[j])
                mx[j] = jnp.max(full, axis=0, keepdims=True)

        def v_step(n, d):
            j, b = vblocks[n]
            accs = vacc.setdefault(n, [None] * NQT)
            ln = j * Dh + d
            kb = kb_sc[kbase + n * Dh + d]
            for t in range(NQT):
                pr = kb * qb_sc[zrow, ln:ln + 1, t * LANES:(t + 1) * LANES]
                accs[t] = pr if accs[t] is None else accs[t] + pr
            if (n * Dh + d + 1) % DS == 0:
                rot[0] = (rot[0] + ROT) % (VR * NQT)
                v = rot[0] % VR
                chain.append(accs[rot[0] // VR][8 * v:8 * v + 8, :])
                if len(chain) > LAG:
                    kb_sc[CH, 0:8, :] = chain.pop(0)
                if fin:
                    kb_sc[CH, 8:16, :] = fin.pop(0)
            if d == Dh - 1:
                st = jnp.concatenate(accs, axis=1)
                s_bufs[j][b * BR:(b + 1) * BR, :] = st
                fold_max(j, jnp.max(st.reshape(VR, 8, TQ), axis=0), m8v, BR)
                fin.extend(m8v[j][:, t * LANES:(t + 1) * LANES] for t in range(NQT))

        def a_piece(j, r0, r1):
            if qm[j] is None:
                qm[j] = jnp.where((row >= j * Dh) & (row < (j + 1) * Dh), qt, 0.0).astype(BF16)
            st = jnp.dot(k_sc[g, r0:r1, :], qm[j], preferred_element_type=F32)
            s_bufs[j][r0:r1, :] = st
            fold_max(j, jnp.max(st.reshape((r1 - r0) // 8, 8, TQ), axis=0), m8, r1 - r0)
            toks.append(st[r1 - r0 - 8:, :])

        def c_chunk(j, c):
            if j == 0 and c == 0 and vblocks:
                s_bufs[0][S:S + 8, :] = toks[-GATE]
                s_bufs[0][S:S + 8, :] = m8v[vblocks[-1][0]]
            p = jnp.exp2(s_bufs[j][pl.ds(zoff + c * TK, TK), :] - mx[j]).astype(BF16)
            pv = jnp.dot(vt_sc[g * HPG + j, :, pl.ds(c * TK, TK)], p, preferred_element_type=F32)
            acc[j] = pv if c == 0 else acc[j] + pv
            if c == NCH - 1:
                outs[j] = acc[j][:Dh, :] * (1.0 / acc[j][Dh:Dh + 1, :])
            pc = j * NCH + c - PG
            if vblocks and 0 <= pc < PN:
                items = kb_items[pc * len(kb_items) // PN:(pc + 1) * len(kb_items) // PN]
                kf_sc[0, NVR:NVR + 16, :] = pv[0:16, 0:GW].astype(BF16)
                make_kb((g + 1) % G, (g + 1) % 2, i, items)

        def gate_task(u, m0, m1):
            gates[(u, m0)] = jnp.dot(xn[m0:m1], w1_ref[:, u * LANES:(u + 1) * LANES], preferred_element_type=F32)

        def up_task(u, m0, m1):
            hg = 0.5 * gates.pop((u, m0))
            up = jnp.dot(xn[m0:m1], w3_ref[:, u * LANES:(u + 1) * LANES], preferred_element_type=F32)
            h_sc[m0:m1, u * LANES:(u + 1) * LANES] = ((hg + hg * jnp.tanh(hg)) * up).astype(BF16)

        P = functools.partial
        main, riders = [], []

        def add(fn, w=0):
            main.append((fn, w))
            riders.append([])

        for u in range(GU0):
            add(P(gate_task, u, 0, TF), WG)
            add(P(up_task, u, 0, TF), WG)
        rs = [xt_ref[:, pl.ds(t0, TF)].astype(F32)]

        def down_range(f0, f1):
            rs[0] = rs[0] + lax.dot_general(w2t_ref[:, f0:f1], h_sc[:, f0:f1], NT, preferred_element_type=F32)
            if f1 < F:
                r_sc[0] = rs[0]

        if DW:
            add(P(down_range, 0, DW * LANES), WD * DW * D // (4 * TK))
        c_list = [(j, c) for j in range(HPG) for c in range(NCH)]
        nxt = 0
        pos = 0
        a_end = []
        for j in range(HPG):
            r0 = vch[j] * VU
            while r0 < S:
                in_win = pos < WIN
                ready = (not in_win and nxt < len(c_list) and c_list[nxt][0] < len(a_end)
                         and pos >= a_end[c_list[nxt][0]] + SK2)
                n = min(PA if ready else TK, S - r0)
                if in_win:
                    n = min(n, WIN - pos)
                add(P(a_piece, j, r0, r0 + n), n * 100 // TK if pos + n <= WIN - GATE * TK + TK else 0)
                r0 += n
                pos += n
                if ready:
                    riders[-1].append(P(c_chunk, *c_list[nxt]))
                    nxt += 1
            a_end.append(pos)
        p0 = len(main)
        for u in range(GU0, NU):
            for m0 in range(0, TF, PGU):
                add(P(gate_task, u, m0, m0 + PGU))
            for m0 in range(0, TF, PGU):
                add(P(up_task, u, m0, m0 + PGU))
        late = [P(c_chunk, *jc) for jc in c_list[nxt:]]
        post = list(range(p0, len(main)))
        nskip = max(0, LSK - (len(late) - NCH))
        post = post[nskip:]
        for n, rd in enumerate(late):
            riders[post[((n + 1) * len(post) - 1) // len(late)]].append(rd)
        vsteps = [(n, d) for n in range(len(vblocks)) for d in range(Dh)]
        NVS = len(vsteps)
        wtot = sum(w for _, w in main)
        cum, done = 0, 0
        for k, (fn, w) in enumerate(main):
            cum += w
            while done < NVS and done * wtot < cum * NVS:
                v_step(*vsteps[done])
                done += 1
            fn()
            for rd in riders[k]:
                rd()
        ot = jnp.concatenate(outs, axis=0).astype(BF16)

        if DW:
            rs[0] = r_sc[zrow]
        down_range(DW * LANES, F)
        r = rs[0]
        at = jnp.dot(wot_sc[g], ot, preferred_element_type=F32)
        for t in range(G):
            cols = slice(t * TF, (t + 1) * TF)
            prev = jnp.where(g == 0, 0.0, acc_sc[i, :, cols]) + jnp.where(g == t, r, 0.0)
            a_t = at[:, cols] + prev
            acc_sc[i, :, cols] = a_t
            o_ref[:, cols] = a_t.astype(o_ref.dtype)

    first = jnp.logical_and(g == 0, i == 0)
    if SCOPE:
        with jax.named_scope("prologue"):
            pl.when(first)(_prologue)
        with jax.named_scope("body"):
            _body()
    else:
        pl.when(first)(_prologue)
        _body()


@jax.jit
def pallas_parallel_sum__softmax_full_mha__glu_gated_swiglu__prompt_kernel(
    A_x: jax.Array,
    A_wqkv: jax.Array,
    A_wo: jax.Array,
    B_x: jax.Array,
    B_w1: jax.Array,
    B_w3: jax.Array,
    B_w2: jax.Array,
):
    B, S, D = A_x.shape
    F = B_w1.shape[1]
    TQ, TC = CFG["TQ"], CFG["TC"]
    G = H // HPG
    Dh = D // H
    GW = HPG * Dh
    BR = 8 * CFG["VR"]
    nkb = 2 * sum(_vchunks(CFG["VC"])) * (VU // BR) * Dh
    xt = A_x.reshape(S, D).T
    w2t = B_w2.T

    ins = (xt, A_wqkv, A_wo, B_w1, B_w3, w2t)
    out = pl.pallas_call(
        functools.partial(_kernel, S=S, D=D, F=F, **CFG),
        grid=(G, S // TQ),
        in_specs=[pl.BlockSpec(memory_space=pl.ANY)] * len(ins),
        out_specs=pl.BlockSpec((D, TQ), lambda g, i: (0, jnp.where(g == G - 1, i, 0))),
        out_shape=jax.ShapeDtypeStruct((D, S), A_x.dtype),
        scratch_shapes=[pltpu.VMEM(a.shape, a.dtype) for a in ins] + [
            pltpu.SemaphoreType.DMA((S // TC + 6,)),
            pltpu.VMEM((D, S), BF16),
            pltpu.VMEM((G, S, GW), BF16),
            pltpu.VMEM((H, HP, S), BF16),
            pltpu.VMEM((D, D), BF16),
            pltpu.VMEM((G, GW, D), BF16),
            pltpu.VMEM((D, D), BF16),
            pltpu.VMEM((G, D, GW), BF16),
            pltpu.VMEM((TQ // G, F), BF16),
            pltpu.VMEM((S // TQ, D, TQ), F32),
            pltpu.VMEM((2, TQ // G, D), BF16),
            pltpu.VMEM((nkb + 2, BR, LANES), F32),
            pltpu.VMEM((2, GW, TQ), F32),
            pltpu.VMEM((HPG, 8, TQ), F32),
            pltpu.VMEM((G, max(_vchunks(CFG["VC"])) * VU + KPAD, GW), BF16),
            pltpu.VMEM((2, D, TQ // G), F32),
        ] + [pltpu.VMEM((S + 8, TQ), F32)] * HPG,
        compiler_params=pltpu.CompilerParams(
            dimension_semantics=("arbitrary", "arbitrary"),
            vmem_limit_bytes=110 * 1024 * 1024,
        ),
    )(*ins)
    return out.T.reshape(B, S, D)
```

```python
import functools
import math

import jax
import jax.numpy as jnp
from jax import lax
import jax.experimental.pallas as pl
import jax.experimental.pallas.tpu as pltpu

H = 16
HP = 32
HPG = 4
LANES = 128
EPS = 1e-5
VU = 64
BR = 16

NT = (((1,), (1,)), ((), ()))
F32 = jnp.float32
BF16 = jnp.bfloat16

CFG = dict(TQ=512, TC=256, TK=128, GU0=10, WIN=5248, VC=3550, DS=3, ROT=3,
           GATE=256, KF32=0, PA=48, SK2=384, PGU=64, LSK=2, LE=1, PG=63, PN=1, MSP=2, AF=1856, NV1=7, LNE=1, SCOPE=0)


def _vchunks(vc):
    return [int(ch) for ch in str(vc).zfill(HPG)]


def _kernel(xt_hbm, wqkv_hbm, wo_hbm, w1_hbm, w3_hbm, w2t_hbm, o_ref,
            xt_ref, wqkv_ref, wo_ref, w1_ref, w3_ref, w2t_ref, sems,
            xnt_sc, k_sc, vt_sc, wkt_sc, wqt_sc, wvt_sc, wot_sc, h_sc, acc_sc, xn_sc, kb_sc, qb_sc, m_sc,
            kf_sc,
            *s_bufs, S, D, F, TQ, TC, TK, GU0, WIN, VC, DS, ROT, GATE, KF32, PA, SK2, PGU, LSK, LE,
            PG, PN, MSP, AF, NV1, LNE, SCOPE):
    Dh = D // H
    G = H // HPG
    GW = HPG * Dh
    NC = S // TC
    NQ = S // TQ
    NS = G * NQ
    TF = TQ // G
    assert TF == LANES
    NU = F // LANES
    NCH = S // TK
    NQT = TQ // LANES
    VR = BR // 8
    qscale = (Dh ** -0.5) * math.log2(math.e)
    vch = _vchunks(VC)
    NBC = VU // BR
    NVR = max(vch) * VU
    vblocks = [(j, b) for j in range(HPG) for b in range(vch[j] * NBC)]
    KBG = len(vblocks) * Dh
    CH = 2 * KBG
    KG = 8 if kf_sc.dtype == F32 else 16
    k_out = pl.program_id(0)
    zrow = k_out >> 8
    P = functools.partial

    TPC = TC // LANES
    NX = S // LANES

    class x_copy:
        def __init__(self, c):
            self.cps = [pltpu.make_async_copy(xt_hbm.at[:, pl.ds(t * LANES, LANES)], xt_ref.at[t], sems.at[t])
                        for t in range(c * TPC, (c + 1) * TPC)]

        def start(self):
            for cp in self.cps:
                cp.start()

        def wait(self):
            for cp in self.cps:
                cp.wait()

    def xnt_chunk(t0):
        return jnp.concatenate([xnt_sc[t0 + t] for t in range(TPC)], axis=1)

    w_copies = [pltpu.make_async_copy(src, dst, sems.at[NX + n]) for n, (src, dst) in enumerate(
        [(wo_hbm, wo_ref), (w1_hbm, w1_ref), (w3_hbm, w3_ref), (w2t_hbm, w2t_ref)])]
    wv_copy = pltpu.make_async_copy(wqkv_hbm.at[:, 2 * D:], wqkv_ref.at[:, 2 * D:], sems.at[NX + 4])
    wqk_copy = pltpu.make_async_copy(wqkv_hbm.at[:, :2 * D], wqkv_ref.at[:, :2 * D], sems.at[NX + 5])

    def layernorm(c):
        for t in range(c * TPC, (c + 1) * TPC):
            x = xt_ref[t].astype(F32)
            mu = jnp.mean(x, axis=0, keepdims=True)
            xc = x - mu
            var = jnp.mean(xc * xc, axis=0, keepdims=True)
            xnt_sc[t] = (xc * lax.rsqrt(var + EPS)).astype(BF16)

    def proj_k(c):
        cols = pl.ds(c * TC, TC)
        kt = jnp.dot(wkt_sc[...], xnt_chunk(c * TPC), preferred_element_type=F32).astype(BF16)
        for gg in range(G):
            kg = kt[gg * GW:(gg + 1) * GW, :].T
            k_sc[gg, cols, :] = kg
            if c * TC < NVR:
                nr = min(TC, NVR - c * TC)
                kf_sc[gg, c * TC:c * TC + nr, :] = kg[:nr, :].astype(kf_sc.dtype)

    def proj_v(c):
        cols = pl.ds(c * TC, TC)
        vt = jnp.dot(wvt_sc[...], xnt_chunk(zrow + c * TPC), preferred_element_type=F32)
        row = lax.broadcasted_iota(jnp.int32, (HP - Dh, TC), 0)
        tail = jnp.where(row == 0, 1.0, 0.0).astype(F32)
        for h in range(H):
            vh = jnp.concatenate([vt[h * Dh:(h + 1) * Dh, :], tail], axis=0)
            vt_sc[h, :, cols] = vh.astype(BF16)

    kb_items = [(j, d) for j in range(HPG) if vch[j] for d in range(Dh)]

    def make_kb(src, gg, slot, part, items):
        kf = {}
        for j, d in items:
            nb = vch[j] * NBC // NQ
            base = slot * KBG + (sum(vch[:j]) * NBC + part * nb) * Dh
            if nb not in kf:
                r0 = part * (nb * BR)
                if not isinstance(part, int):
                    r0 = pl.multiple_of(r0, nb * BR)
                kf[nb] = src[gg, pl.ds(r0, nb * BR), :].astype(F32)
            kb = jnp.broadcast_to(kf[nb][:, j * Dh + d:j * Dh + d + 1], (nb * BR, LANES))
            for b in range(nb):
                kb_sc[base + b * Dh + d] = kb[b * BR:(b + 1) * BR, :]

    def q_tile(gg, ii, t):
        qb_sc[0, :, t * LANES:(t + 1) * LANES] = qscale * jnp.dot(
            wqt_sc[gg], xnt_sc[ii * NQT + t], preferred_element_type=F32)

    def _prologue():
        wv_copy.start()
        for c in range(NC):
            x_copy(c).start()
        wqk_copy.start()
        for cp in w_copies:
            cp.start()
        acc_sc[...] = jnp.zeros(acc_sc.shape, F32)
        wv_copy.wait()
        wvt_sc[...] = wqkv_ref[:, 2 * D:].T
        x_copy(0).wait()
        layernorm(0)
        x_copy(1).wait()
        waited, normed = 2, 1
        for c in range(NV1):
            if c + 1 >= waited:
                nxt = min(NC, 2 * waited)
                for cc in range(waited, nxt):
                    x_copy(cc).wait()
                waited = nxt
            if c == NV1 - 1:
                wqk_copy.wait()
                w_copies[0].wait()
            proj_v(c)
            upto = NC if c == NV1 - 2 and LNE else min(c + 2, NC)
            for cc in range(normed, upto):
                layernorm(cc)
            normed = max(normed, upto)
        wqkt = wqkv_ref[:, :2 * D].T
        wkt_sc[...] = wqkt[D:, :]
        for gg in range(G):
            wqt_sc[gg] = wqkt[gg * GW:(gg + 1) * GW, :]
        kb_first = -(-NVR // TC)
        for c in range(NC):
            proj_k(c)
            if normed < NC:
                layernorm(normed)
                normed += 1
            if c == 1:
                for gg in range(G):
                    wot_sc[gg] = wo_ref[gg * GW:(gg + 1) * GW, :].T
            if kb_first <= c < kb_first + NQ:
                make_kb(k_sc, 0, 0, c - kb_first, kb_items)
        for t in range(NQT):
            q_tile(0, 0, t)
        for c in range(NV1, NC):
            proj_v(c)
        for cp in w_copies[1:]:
            cp.wait()

    def closing_tasks(s, acc):
        gp = s // NQ
        ip = s % NQ
        MS = D // MSP
        st = {}

        def down(m):
            rows = slice(m * MS, (m + 1) * MS)
            st[m] = xt_ref[ip * G + gp, rows, :].astype(F32) + lax.dot_general(
                w2t_ref[rows, :], h_sc[...], NT, preferred_element_type=F32)

        def outp(m):
            rows = slice(m * MS, (m + 1) * MS)
            if "ot" not in st:
                outs = [a[:Dh, :] * (1.0 / a[Dh:Dh + 1, :]) for a in acc]
                st["ot"] = jnp.concatenate(outs, axis=0).astype(BF16)
            at = jnp.dot(wot_sc[gp, rows, :], st["ot"], preferred_element_type=F32)
            r = st.pop(m)
            for t in range(G):
                cols = slice(t * TF, (t + 1) * TF)
                a_t = at[:, cols] + (acc_sc[ip * G + t, rows, :] + jnp.where(gp == t, r, 0.0))
                acc_sc[ip * G + t, rows, :] = a_t
                o_ref[rows, cols] = a_t.astype(o_ref.dtype)

        return [fn for m in range(MSP) for fn in (P(down, m), P(outp, m))]

    def _body(s):
        g = s // NQ
        i = s % NQ
        zoff = pl.multiple_of(zrow * TK, TK)
        sn = (s + 1) % NS
        g2, i2 = sn // NQ, sn % NQ
        gn = (g + 1) % G
        win = WIN
        xn_sc[0] = xnt_sc[i * G + g].T
        xn = xn_sc[zrow]
        row = lax.broadcasted_iota(jnp.int32, (GW, TQ), 0)
        qrow = zrow

        qm = [None] * HPG
        m8 = [None] * HPG
        m8v = [None] * HPG
        mx = [None] * HPG
        acc = [None] * HPG
        left = [S] * HPG
        lefta = [S - vch[j] * VU for j in range(HPG)]
        chain, fin, toks, cnt = [], [], [], [0]
        vacc, gates = {}, {}
        kbase = (g % 2) * KBG + zrow

        def fold_max(j, cm, mm, nrows):
            mm[j] = cm if mm[j] is None else jnp.maximum(mm[j], cm)
            left[j] -= nrows
            if mm is m8:
                lefta[j] -= nrows
                if lefta[j] == 0 and vch[j]:
                    m_sc[j] = m8[j]
            if left[j] == 0:
                full = m8[j] if m8v[j] is None else jnp.maximum(m_sc[zrow + j], m8v[j])
                mx[j] = jnp.max(full, axis=0, keepdims=True)

        def v_step(n, d):
            j, b = vblocks[n]
            accs = vacc.setdefault(n, [None] * NQT)
            ln = j * Dh + d
            kb = kb_sc[kbase + n * Dh + d]
            for t in range(NQT):
                pr = kb * qb_sc[qrow, ln:ln + 1, t * LANES:(t + 1) * LANES]
                accs[t] = pr if accs[t] is None else accs[t] + pr
            cnt[0] += 1
            if cnt[0] % DS == 0:
                rot = (cnt[0] // DS * ROT) % (VR * NQT)
                chain.append(accs[rot // VR][8 * (rot % VR):8 * (rot % VR) + 8, :])
                if len(chain) > 1:
                    kb_sc[CH, 0:8, :] = chain.pop(0)
                if fin:
                    kb_sc[CH, 8:16, :] = fin.pop(0)
            if d == Dh - 1:
                st = jnp.concatenate(accs, axis=1)
                s_bufs[j][b * BR:(b + 1) * BR, :] = st
                fold_max(j, jnp.max(st.reshape(VR, 8, TQ), axis=0), m8v, BR)
                fin.extend(m8v[j][:, t * LANES:(t + 1) * LANES] for t in range(NQT))

        def a_piece(j, r0, r1):
            if qm[j] is None:
                qm[j] = jnp.where((row >= j * Dh) & (row < (j + 1) * Dh), qb_sc[qrow], 0.0).astype(BF16)
            st = jnp.dot(k_sc[g, r0:r1, :], qm[j], preferred_element_type=F32)
            s_bufs[j][r0:r1, :] = st
            fold_max(j, jnp.max(st.reshape((r1 - r0) // 8, 8, TQ), axis=0), m8, r1 - r0)
            toks.append((r1 - r0, st[r1 - r0 - 8:, :]))

        def c_chunk(j, c):
            if j == 0 and c == 0:
                back, k = 0, len(toks) - 1
                while back < GATE:
                    back += toks[k][0]
                    k -= 1
                s_bufs[0][S:S + 8, :] = toks[k][1]
                s_bufs[0][S:S + 8, :] = m8v[vblocks[-1][0]]
            p = jnp.exp2(s_bufs[j][pl.ds(zoff + c * TK, TK), :] - mx[j]).astype(BF16)
            pv = jnp.dot(vt_sc[g * HPG + j, :, pl.ds(c * TK, TK)], p, preferred_element_type=F32)
            acc[j] = pv if c == 0 else acc[j] + pv
            pc = j * NCH + c - PG
            if 0 <= pc < PN:
                items = kb_items[pc * len(kb_items) // PN:(pc + 1) * len(kb_items) // PN]
                kf_sc[0, NVR:NVR + KG, :] = pv[0:KG, 0:GW].astype(kf_sc.dtype)
                make_kb(kf_sc, gn + zrow, gn % 2, i, items)

        def gate_task(u, m0, m1):
            gates[(u, m0)] = jnp.dot(xn[m0:m1], w1_ref[:, u * LANES:(u + 1) * LANES], preferred_element_type=F32)

        def up_task(u, m0, m1):
            hg = 0.5 * gates.pop((u, m0))
            up = jnp.dot(xn[m0:m1], w3_ref[:, u * LANES:(u + 1) * LANES], preferred_element_type=F32)
            h_sc[m0:m1, u * LANES:(u + 1) * LANES] = ((hg + hg * jnp.tanh(hg)) * up).astype(BF16)

        main, riders = [], []

        def add(fn):
            main.append(fn)
            riders.append([])

        if AF:
            add(P(a_piece, 0, vch[0] * VU, vch[0] * VU + AF))
        for u in range(GU0):
            add(P(gate_task, u, 0, TF))
            add(P(up_task, u, 0, TF))
        c_list = [(j, c) for j in range(HPG) for c in range(NCH)]
        nxt = 0
        pos = AF
        a_end = []
        nwin = None
        for j in range(HPG):
            r0 = vch[j] * VU + (AF if j == 0 else 0)
            while r0 < S:
                in_win = pos < win
                if not in_win and nwin is None:
                    nwin = len(main)
                ready = (not in_win and nxt < len(c_list) and c_list[nxt][0] < len(a_end)
                         and pos >= a_end[c_list[nxt][0]] + SK2)
                n = min(PA if ready else TK, S - r0)
                if in_win:
                    n = min(n, win - pos)
                add(P(a_piece, j, r0, r0 + n))
                r0 += n
                pos += n
                if ready:
                    riders[-1].append(P(c_chunk, *c_list[nxt]))
                    nxt += 1
            a_end.append(pos)
        p0 = len(main)
        for t in range(NQT):
            add(P(q_tile, g2, i2, t))
        for u in range(GU0, NU):
            for m0 in range(0, TF, PGU):
                add(P(gate_task, u, m0, m0 + PGU))
            for m0 in range(0, TF, PGU):
                add(P(up_task, u, m0, m0 + PGU))
        late = [P(c_chunk, *jc) for jc in c_list[nxt:]]
        post = list(range(p0, len(main)))
        nskip = max(0, LSK - (len(late) - NCH))
        post = post[nskip:len(post) - LE]
        for n, rd in enumerate(late):
            riders[post[((n + 1) * len(post) - 1) // len(late)]].append(rd)

        vsteps = [(n, d) for n in range(len(vblocks)) for d in range(Dh)]
        for k, fn in enumerate(main):
            if k < nwin:
                for n, d in vsteps[k * len(vsteps) // nwin:(k + 1) * len(vsteps) // nwin]:
                    v_step(n, d)
            fn()
            for rd in riders[k]:
                rd()
        for fn in closing_tasks(s, acc):
            fn()

    def scoped(name, fn):
        def run(*a):
            if SCOPE:
                with jax.named_scope(name):
                    fn(*a)
            else:
                fn(*a)
        return run

    def step(s, carry):
        scoped("body", _body)(s)
        return carry

    pl.when(k_out == 0)(scoped("prologue", _prologue))
    hi = NS - NQ + 1 + k_out
    lax.fori_loop(jnp.where(k_out == 0, 0, hi - 1), hi, step, 0)


@jax.jit
def pallas_parallel_sum__softmax_full_mha__glu_gated_swiglu__prompt_kernel(
    A_x: jax.Array,
    A_wqkv: jax.Array,
    A_wo: jax.Array,
    B_x: jax.Array,
    B_w1: jax.Array,
    B_w3: jax.Array,
    B_w2: jax.Array,
):
    B, S, D = A_x.shape
    F = B_w1.shape[1]
    TQ, TC = CFG["TQ"], CFG["TC"]
    G = H // HPG
    Dh = D // H
    GW = HPG * Dh
    NQ = S // TQ
    vch = _vchunks(CFG["VC"])
    nkb = 2 * sum(vch) * (VU // BR) * Dh + 2
    xt = A_x.reshape(S, D).T
    w2t = B_w2.T

    ins = (xt, A_wqkv, A_wo, B_w1, B_w3, w2t)
    out = pl.pallas_call(
        functools.partial(_kernel, S=S, D=D, F=F, **CFG),
        grid=(NQ,),
        in_specs=[pl.BlockSpec(memory_space=pl.ANY)] * len(ins),
        out_specs=pl.BlockSpec((D, TQ), lambda k: (0, k)),
        out_shape=jax.ShapeDtypeStruct((D, S), A_x.dtype),
        scratch_shapes=[pltpu.VMEM((S // LANES, D, LANES), BF16)] + [pltpu.VMEM(a.shape, a.dtype) for a in ins[1:]] + [
            pltpu.SemaphoreType.DMA((S // LANES + 6,)),
            pltpu.VMEM((S // LANES, D, LANES), BF16),
            pltpu.VMEM((G, S, GW), BF16),
            pltpu.VMEM((H, HP, S), BF16),
            pltpu.VMEM((D, D), BF16),
            pltpu.VMEM((G, GW, D), BF16),
            pltpu.VMEM((D, D), BF16),
            pltpu.VMEM((G, D, GW), BF16),
            pltpu.VMEM((TQ // G, F), BF16),
            pltpu.VMEM((NQ * G, D, TQ // G), F32),
            pltpu.VMEM((2, TQ // G, D), BF16),
            pltpu.VMEM((nkb, BR, LANES), F32),
            pltpu.VMEM((2, GW, TQ), F32),
            pltpu.VMEM((HPG, 8, TQ), F32),
            pltpu.VMEM((G, max(vch) * VU + 64, GW), F32 if CFG["KF32"] else BF16),
        ] + [pltpu.VMEM((S + 8, TQ), F32)] * HPG,
        compiler_params=pltpu.CompilerParams(
            dimension_semantics=("arbitrary",),
            vmem_limit_bytes=110 * 1024 * 1024,
        ),
    )(*ins)
    return out.T.reshape(B, S, D)
```

```python
import functools
import math

import jax
import jax.numpy as jnp
from jax import lax
import jax.experimental.pallas as pl
import jax.experimental.pallas.tpu as pltpu

H = 16
HP = 32
HPG = 4
LANES = 128
EPS = 1e-5
VU = 64
BR = 16

NT = (((1,), (1,)), ((), ()))
F32 = jnp.float32
BF16 = jnp.bfloat16

CFG = dict(TQ=512, TC=256, TK=128, GU0=10, WIN=5248, VC=3550, DS=3, ROT=5,
           GATE=256, KF32=0, PA=48, SK2=384, PGU=64, LSK=2, LE=0, PG=63, PN=1, PF=45, PR=192, AF=1856, NV1=7, ND0=14, ND1=14, ND2=14, LNE=1, NOBC=1, SCOPE=0)


def _vchunks(vc):
    return [int(ch) for ch in str(vc).zfill(HPG)]


def _kernel(xt_hbm, wqkv_hbm, wo_hbm, w1_hbm, w3_hbm, w2t_hbm, o_hbm,
            xt_ref, wqkv_ref, wo_ref, w1_ref, w3_ref, w2t_ref, sems,
            xnt_sc, k_sc, vt_sc, wkt_sc, wqt_sc, wvt_sc, wot_sc, h_sc, acc_sc, xn_sc, kb_sc, qb_sc, m_sc,
            kf_sc, o_ref, osems,
            *s_bufs, S, D, F, TQ, TC, TK, GU0, WIN, VC, DS, ROT, GATE, KF32, PA, SK2, PGU, LSK, LE,
            PG, PN, PF, PR, AF, NV1, ND0, ND1, ND2, LNE, NOBC, SCOPE):
    Dh = D // H
    G = H // HPG
    GW = HPG * Dh
    NC = S // TC
    NQ = S // TQ
    NS = G * NQ
    TF = TQ // G
    assert TF == LANES
    NU = F // LANES
    NCH = S // TK
    NQT = TQ // LANES
    VR = BR // 8
    qscale = (Dh ** -0.5) * math.log2(math.e)
    vch = _vchunks(VC)
    NBC = VU // BR
    NVR = max(vch) * VU
    vblocks = [(j, b) for j in range(HPG) for b in range(vch[j] * NBC)]
    KBG = len(vblocks) * Dh
    CH = 2 * KBG
    KG = 8 if kf_sc.dtype == F32 else 16
    phase = pl.program_id(0)
    zrow = phase >> 8
    P = functools.partial

    TPC = TC // LANES
    NX = (NC - 1).bit_length() + 1

    def x_copy(c):
        return pltpu.make_async_copy(xt_hbm.at[:, pl.ds(c * TC, TC)], xt_ref.at[:, pl.ds(c * TC, TC)],
                                     sems.at[c.bit_length()])

    def xnt_chunk(t0):
        return jnp.concatenate([xnt_sc[t0 + t] for t in range(TPC)], axis=1)

    w_copies = [pltpu.make_async_copy(src, dst, sems.at[NX + n]) for n, src, dst in
                [(0, wo_hbm, wo_ref), (1, w1_hbm, w1_ref), (1, w3_hbm, w3_ref), (1, w2t_hbm, w2t_ref)]]
    wv_copy = pltpu.make_async_copy(wqkv_hbm.at[:, 2 * D:], wqkv_ref.at[:, 2 * D:], sems.at[NX + 2])
    wqk_copy = pltpu.make_async_copy(wqkv_hbm.at[:, :2 * D], wqkv_ref.at[:, :2 * D], sems.at[NX])

    def layernorm(c):
        for t in range(c * TPC, (c + 1) * TPC):
            x = xt_ref[:, t * LANES:(t + 1) * LANES].astype(F32)
            mu = jnp.mean(x, axis=0, keepdims=True)
            xc = x - mu
            var = jnp.mean(xc * xc, axis=0, keepdims=True)
            xnt_sc[t] = (xc * lax.rsqrt(var + EPS)).astype(BF16)

    def proj_k(c):
        cols = pl.ds(c * TC, TC)
        kt = jnp.dot(wkt_sc[...], xnt_chunk(c * TPC), preferred_element_type=F32).astype(BF16)
        for gg in range(G):
            kg = kt[gg * GW:(gg + 1) * GW, :].T
            k_sc[gg, cols, :] = kg
            if c * TC < NVR:
                nr = min(TC, NVR - c * TC)
                kf_sc[gg, c * TC:c * TC + nr, :] = kg[:nr, :].astype(kf_sc.dtype)

    def proj_v(c):
        cols = pl.ds(c * TC, TC)
        vt = jnp.dot(wvt_sc[...], xnt_chunk(zrow + c * TPC), preferred_element_type=F32)
        row = lax.broadcasted_iota(jnp.int32, (HP - Dh, TC), 0)
        tail = jnp.where(row == 0, 1.0, 0.0).astype(F32)
        for h in range(H):
            vh = jnp.concatenate([vt[h * Dh:(h + 1) * Dh, :], tail], axis=0)
            vt_sc[h, :, cols] = vh.astype(BF16)

    kb_items = [(j, d) for j in range(HPG) if vch[j] for d in range(Dh)]

    def make_kb(src, gg, slot, part, items):
        kf = {}
        for j, d in items:
            nb = vch[j] * NBC // NQ
            base = slot * KBG + (sum(vch[:j]) * NBC + part * nb) * Dh
            if nb not in kf:
                r0 = part * (nb * BR)
                if not isinstance(part, int):
                    r0 = pl.multiple_of(r0, nb * BR)
                kf[nb] = src[gg, pl.ds(r0, nb * BR), :].astype(F32)
            kb = jnp.broadcast_to(kf[nb][:, j * Dh + d:j * Dh + d + 1], (nb * BR, LANES))
            for b in range(nb):
                kb_sc[base + b * Dh + d] = kb[b * BR:(b + 1) * BR, :]

    def q_tile(gg, ii, t):
        qb_sc[0, :, t * LANES:(t + 1) * LANES] = qscale * jnp.dot(
            wqt_sc[gg], xnt_sc[ii * NQT + t], preferred_element_type=F32)

    def _prologue():
        order = [wv_copy] + [x_copy(c) for c in range(NC)] + [wqk_copy] + w_copies
        for cp in order[:ND0]:
            cp.start()
        na = acc_sc.shape[0]
        acc_sc[:na // 2] = jnp.zeros((na // 2,) + acc_sc.shape[1:], F32)
        for cp in order[ND0:ND1]:
            cp.start()
        acc_sc[na // 2:] = jnp.zeros((na // 2,) + acc_sc.shape[1:], F32)
        for cp in order[ND1:ND2]:
            cp.start()
        wv_copy.wait()
        for cp in order[ND2:]:
            cp.start()
        wvt_sc[...] = wqkv_ref[:, 2 * D:].T
        x_copy(0).wait()
        layernorm(0)
        x_copy(1).wait()
        waited, normed = 2, 1
        for c in range(NV1):
            if c + 1 >= waited:
                nxt = min(NC, 2 * waited)
                for cc in range(waited, nxt):
                    x_copy(cc).wait()
                waited = nxt
            if c == NV1 - 1:
                wqk_copy.wait()
                w_copies[0].wait()
            proj_v(c)
            upto = NC if c == NV1 - 2 and LNE else min(c + 2, NC)
            for cc in range(normed, upto):
                layernorm(cc)
            normed = max(normed, upto)
        wqkt = wqkv_ref[:, :2 * D].T
        wkt_sc[...] = wqkt[D:, :]
        for gg in range(G):
            wqt_sc[gg] = wqkt[gg * GW:(gg + 1) * GW, :]
        kb_first = -(-NVR // TC)
        for c in range(NC):
            proj_k(c)
            if normed < NC:
                layernorm(normed)
                normed += 1
            if c == 1:
                for gg in range(G):
                    wot_sc[gg] = wo_ref[gg * GW:(gg + 1) * GW, :].T
            if kb_first <= c < kb_first + NQ:
                make_kb(k_sc, 0, 0, c - kb_first, kb_items)
        for t in range(NQT):
            q_tile(0, 0, t)
        for c in range(NV1, NC):
            proj_v(c)
        for cp in w_copies[1:]:
            cp.wait()

    HM = D // 2
    o_parts = [(0, HM, 0, TQ), (HM, D, 0, TQ - TF), (HM, D, TQ - TF, TQ)]

    def o_copy(ii, k):
        r0, r1, c0, c1 = o_parts[k]
        q0 = ii * TQ + c0
        if not isinstance(ii, int):
            q0 = pl.multiple_of(q0, LANES)
        return pltpu.make_async_copy(o_ref.at[ii, r0:r1, c0:c1], o_hbm.at[r0:r1, pl.ds(q0, c1 - c0)], osems.at[0])

    def closing(s, acc, rider):
        gp = s // NQ
        ip = s % NQ
        tp = pl.multiple_of((ip * G + gp) * TF, TF)

        def down(rows):
            return xt_ref[rows, pl.ds(tp, TF)].astype(F32) + lax.dot_general(
                w2t_ref[rows, :], h_sc[...], NT, preferred_element_type=F32)

        lo, hi = slice(0, HM), slice(HM, D)
        pl.when(s > NS - NQ)(lambda: o_copy(ip - 1, 2).start())
        r = down(lo)
        outs = [a[:Dh, :] * (1.0 / a[Dh:Dh + 1, :]) for a in acc]
        ot = jnp.concatenate(outs, axis=0).astype(BF16)
        for k, rows in enumerate((lo, hi)):
            at = jnp.dot(wot_sc[gp, rows, :], ot, preferred_element_type=F32)
            for t in range(G):
                cols = slice(t * TF, (t + 1) * TF)
                prev = acc_sc[ip * G + t, rows, :]
                if k == 0:
                    prev = prev + jnp.where(gp == t, r, 0.0)
                a_t = at[:, cols] + prev
                acc_sc[ip * G + t, rows, :] = a_t
                if k == 0 or t < G - 1:
                    o_ref[ip, rows, cols] = a_t.astype(o_ref.dtype)
            pl.when(gp == G - 1)(lambda k=k: o_copy(ip, k).start())
        rider(at[PR:])
        a_t = acc_sc[ip * G + gp, hi, :] + down(hi)
        acc_sc[ip * G + gp, hi, :] = a_t
        o_ref[ip, hi, TQ - TF:] = a_t.astype(o_ref.dtype)

    def _body(s):
        g = s // NQ
        i = s % NQ
        zoff = pl.multiple_of(zrow * TK, TK)
        sn = (s + 1) % NS
        g2, i2 = sn // NQ, sn % NQ
        gn = (g + 1) % G
        win = WIN
        xn_sc[0] = xnt_sc[i * G + g].T
        xn = xn_sc[zrow]
        row = lax.broadcasted_iota(jnp.int32, (GW, TQ), 0)
        qrow = zrow

        qm = [None] * HPG
        m8 = [None] * HPG
        m8v = [None] * HPG
        mx = [None] * HPG
        acc = [None] * HPG
        left = [S] * HPG
        lefta = [S - vch[j] * VU for j in range(HPG)]
        chain, fin, toks, cnt = [], [], [], [0]
        vacc, gates = {}, {}
        kbase = (g % 2) * KBG + zrow

        def fold_max(j, cm, mm, nrows):
            mm[j] = cm if mm[j] is None else jnp.maximum(mm[j], cm)
            left[j] -= nrows
            if mm is m8:
                lefta[j] -= nrows
                if lefta[j] == 0 and vch[j]:
                    m_sc[j] = m8[j]
            if left[j] == 0:
                full = m8[j] if m8v[j] is None else jnp.maximum(m_sc[zrow + j], m8v[j])
                mx[j] = jnp.max(full, axis=0, keepdims=True)

        def v_step(n, d):
            j, b = vblocks[n]
            accs = vacc.setdefault(n, [None] * NQT)
            ln = j * Dh + d
            kb = kb_sc[kbase + n * Dh + d]
            for t in range(NQT):
                pr = kb * qb_sc[qrow, ln:ln + 1, t * LANES:(t + 1) * LANES]
                accs[t] = pr if accs[t] is None else accs[t] + pr
            cnt[0] += 1
            if cnt[0] % DS == 0:
                rot = (cnt[0] // DS * ROT) % (VR * NQT)
                chain.append(accs[rot // VR][8 * (rot % VR):8 * (rot % VR) + 8, :])
                if len(chain) > 1:
                    kb_sc[CH, 0:8, :] = chain.pop(0)
                if fin:
                    kb_sc[CH, 8:16, :] = fin.pop(0)
            if d == Dh - 1:
                st = jnp.concatenate(accs, axis=1)
                s_bufs[j][b * BR:(b + 1) * BR, :] = st
                fold_max(j, jnp.max(st.reshape(VR, 8, TQ), axis=0), m8v, BR)
                fin.extend(m8v[j][:, t * LANES:(t + 1) * LANES] for t in range(NQT))

        def a_piece(j, r0, r1):
            if qm[j] is None:
                qm[j] = jnp.where((row >= j * Dh) & (row < (j + 1) * Dh), qb_sc[qrow], 0.0).astype(BF16)
            st = jnp.dot(k_sc[g, r0:r1, :], qm[j], preferred_element_type=F32)
            s_bufs[j][r0:r1, :] = st
            fold_max(j, jnp.max(st.reshape((r1 - r0) // 8, 8, TQ), axis=0), m8, r1 - r0)
            toks.append((r1 - r0, st[r1 - r0 - 8:, :]))

        n1 = len(kb_items) * PF // 100

        def next_kb(items, tok):
            if items:
                kf_sc[0, NVR:NVR + KG, :] = tok[0:KG, 0:GW].astype(kf_sc.dtype)
                make_kb(kf_sc, gn + zrow, gn % 2, i, items)

        def c_chunk(j, c):
            if j == 0 and c == 0:
                back, k = 0, len(toks) - 1
                while back < GATE:
                    back += toks[k][0]
                    k -= 1
                s_bufs[0][S:S + 8, :] = toks[k][1]
                s_bufs[0][S:S + 8, :] = m8v[vblocks[-1][0]]
            p = jnp.exp2(s_bufs[j][pl.ds(zoff + c * TK, TK), :] - mx[j]).astype(BF16)
            pv = jnp.dot(vt_sc[g * HPG + j, :, pl.ds(c * TK, TK)], p, preferred_element_type=F32)
            acc[j] = pv if c == 0 else acc[j] + pv
            pc = j * NCH + c - PG
            if 0 <= pc < PN:
                next_kb(kb_items[pc * n1 // PN:(pc + 1) * n1 // PN], pv)

        def gate_task(u, m0, m1):
            gates[(u, m0)] = jnp.dot(xn[m0:m1], w1_ref[:, u * LANES:(u + 1) * LANES], preferred_element_type=F32)

        def up_task(u, m0, m1):
            hg = 0.5 * gates.pop((u, m0))
            up = jnp.dot(xn[m0:m1], w3_ref[:, u * LANES:(u + 1) * LANES], preferred_element_type=F32)
            h_sc[m0:m1, u * LANES:(u + 1) * LANES] = ((hg + hg * jnp.tanh(hg)) * up).astype(BF16)

        main, riders = [], []

        def add(fn):
            main.append(fn)
            riders.append([])

        if AF:
            add(P(a_piece, 0, vch[0] * VU, vch[0] * VU + AF))
        for u in range(GU0):
            add(P(gate_task, u, 0, TF))
            add(P(up_task, u, 0, TF))
        c_list = [(j, c) for j in range(HPG) for c in range(NCH)]
        nxt = 0
        pos = AF
        a_end = []
        nwin = None
        for j in range(HPG):
            r0 = vch[j] * VU + (AF if j == 0 else 0)
            while r0 < S:
                in_win = pos < win
                if not in_win and nwin is None:
                    nwin = len(main)
                ready = (not in_win and nxt < len(c_list) and c_list[nxt][0] < len(a_end)
                         and pos >= a_end[c_list[nxt][0]] + SK2)
                n = min(PA if ready else TK, S - r0)
                if in_win:
                    n = min(n, win - pos)
                add(P(a_piece, j, r0, r0 + n))
                r0 += n
                pos += n
                if ready:
                    riders[-1].append(P(c_chunk, *c_list[nxt]))
                    nxt += 1
            a_end.append(pos)
        p0 = len(main)
        for t in range(NQT):
            add(P(q_tile, g2, i2, t))
        for u in range(GU0, NU):
            for m0 in range(0, TF, PGU):
                add(P(gate_task, u, m0, m0 + PGU))
            for m0 in range(0, TF, PGU):
                add(P(up_task, u, m0, m0 + PGU))
        late = [P(c_chunk, *jc) for jc in c_list[nxt:]]
        post = list(range(p0, len(main)))
        nskip = max(0, LSK - (len(late) - NCH))
        post = post[nskip:len(post) - LE]
        for n, rd in enumerate(late):
            riders[post[((n + 1) * len(post) - 1) // len(late)]].append(rd)

        vsteps = [(n, d) for n in range(len(vblocks)) for d in range(Dh)]
        for k, fn in enumerate(main):
            if k < nwin:
                for n, d in vsteps[k * len(vsteps) // nwin:(k + 1) * len(vsteps) // nwin]:
                    v_step(n, d)
            fn()
            for rd in riders[k]:
                rd()
        closing(s, acc, P(next_kb, kb_items[n1:]))

    def scoped(name, fn):
        def run(*a):
            if SCOPE:
                with jax.named_scope(name):
                    fn(*a)
            else:
                fn(*a)
        return run

    def step(s, carry):
        scoped("body", _body)(s)
        return carry

    @pl.when(phase == 0)
    def _():
        scoped("prologue", _prologue)()
        lax.fori_loop(0, NS, step, 0)
        o_copy(NQ - 1, 2).start()

    @pl.when(phase == 1)
    def _():
        for ii in range(NQ):
            for k in range(len(o_parts)):
                o_copy(ii, k).wait()


@jax.jit
def pallas_parallel_sum__softmax_full_mha__glu_gated_swiglu__prompt_kernel(
    A_x: jax.Array,
    A_wqkv: jax.Array,
    A_wo: jax.Array,
    B_x: jax.Array,
    B_w1: jax.Array,
    B_w3: jax.Array,
    B_w2: jax.Array,
):
    B, S, D = A_x.shape
    F = B_w1.shape[1]
    TQ, TC = CFG["TQ"], CFG["TC"]
    G = H // HPG
    Dh = D // H
    GW = HPG * Dh
    NQ = S // TQ
    vch = _vchunks(CFG["VC"])
    nkb = 2 * sum(vch) * (VU // BR) * Dh + 2
    xt = A_x.reshape(S, D).T
    w2t = B_w2.T

    ins = (xt, A_wqkv, A_wo, B_w1, B_w3, w2t)
    out = pl.pallas_call(
        functools.partial(_kernel, S=S, D=D, F=F, **CFG),
        grid=(2,),
        in_specs=[pl.BlockSpec(memory_space=pl.ANY)] * len(ins),
        out_specs=pl.BlockSpec(memory_space=pl.ANY),
        out_shape=jax.ShapeDtypeStruct((D, S), A_x.dtype),
        scratch_shapes=[pltpu.VMEM(a.shape, a.dtype) for a in ins] + [
            pltpu.SemaphoreType.DMA(((S // TC - 1).bit_length() + 4,)),
            pltpu.VMEM((S // LANES, D, LANES), BF16),
            pltpu.VMEM((G, S, GW), BF16),
            pltpu.VMEM((H, HP, S), BF16),
            pltpu.VMEM((D, D), BF16),
            pltpu.VMEM((G, GW, D), BF16),
            pltpu.VMEM((D, D), BF16),
            pltpu.VMEM((G, D, GW), BF16),
            pltpu.VMEM((TQ // G, F), BF16),
            pltpu.VMEM((NQ * G, D, TQ // G), F32),
            pltpu.VMEM((2, TQ // G, D), BF16),
            pltpu.VMEM((nkb, BR, LANES), F32),
            pltpu.VMEM((2, GW, TQ), F32),
            pltpu.VMEM((HPG, 8, TQ), F32),
            pltpu.VMEM((G, max(vch) * VU + 64, GW), F32 if CFG["KF32"] else BF16),
            pltpu.VMEM((NQ, D, TQ), BF16),
            pltpu.SemaphoreType.DMA((1,)),
        ] + [pltpu.VMEM((S + 8, TQ), F32)] * HPG,
        compiler_params=pltpu.CompilerParams(
            dimension_semantics=("arbitrary",),
            vmem_limit_bytes=110 * 1024 * 1024,
            disable_bounds_checks=bool(CFG["NOBC"]),
        ),
    )(*ins)
    return out.T.reshape(B, S, D)
```

```python
import functools
import math

import jax
import jax.numpy as jnp
from jax import lax
import jax.experimental.pallas as pl
import jax.experimental.pallas.tpu as pltpu

H = 16
HP = 32
HPG = 4
LANES = 128
EPS = 1e-5

TQ = 512
TC = 256
TK = 128
VU = 64
BR = 16
VUNITS = (3, 5, 5, 0)

GU0 = 10
WIN = 5248
DS = 3
ROT = 5
GATE = 256
PA = 48
PGU = 64
SETTLE = 384
KB_EARLY = 45
KB_ROW = 192

NT = (((1,), (1,)), ((), ()))
F32 = jnp.float32
BF16 = jnp.bfloat16


def _kernel(xt_hbm, wqkv_hbm, wo_hbm, w1_hbm, w3_hbm, w2t_hbm, o_hbm,
            xt_ref, wqkv_ref, wo_ref, w1_ref, w3_ref, w2t_ref, sems,
            xnt_sc, k_sc, vt_sc, wkt_sc, wqt_sc, wvt_sc, wot_sc, h_sc, acc_sc, xn_sc, kb_sc, qb_sc, m_sc,
            kf_sc, o_ref, osems, *s_bufs, S, D, F):
    Dh = D // H
    G = H // HPG
    GW = HPG * Dh
    NC = S // TC
    NQ = S // TQ
    NS = G * NQ
    TF = TQ // G
    NU = F // LANES
    NCH = S // TK
    NQT = TQ // LANES
    TPC = TC // LANES
    VR = BR // 8
    NBC = VU // BR
    NVR = max(VUNITS) * VU
    vblocks = [(j, b) for j in range(HPG) for b in range(VUNITS[j] * NBC)]
    quarter = [VUNITS[j] * NBC // NQ for j in range(HPG)]
    kb_items = [(j, d) for j in range(HPG) if VUNITS[j] for d in range(Dh)]
    KBG = len(vblocks) * Dh
    CH = 2 * KBG
    qscale = (Dh ** -0.5) * math.log2(math.e)
    assert TF == LANES and NBC == NQ
    phase = pl.program_id(0)
    zero = phase >> 8
    P = functools.partial

    NX = (NC - 1).bit_length() + 1

    def x_copy(c):
        return pltpu.make_async_copy(xt_hbm.at[:, pl.ds(c * TC, TC)], xt_ref.at[:, pl.ds(c * TC, TC)],
                                     sems.at[c.bit_length()])

    wv_copy = pltpu.make_async_copy(wqkv_hbm.at[:, 2 * D:], wqkv_ref.at[:, 2 * D:], sems.at[NX + 2])
    wqk_copy = pltpu.make_async_copy(wqkv_hbm.at[:, :2 * D], wqkv_ref.at[:, :2 * D], sems.at[NX])
    wo_copy = pltpu.make_async_copy(wo_hbm, wo_ref, sems.at[NX])
    ffn_copies = [pltpu.make_async_copy(src, dst, sems.at[NX + 1])
                  for src, dst in [(w1_hbm, w1_ref), (w3_hbm, w3_ref), (w2t_hbm, w2t_ref)]]

    HM = D // 2
    o_parts = [(0, HM, 0, TQ), (HM, D, 0, TQ - TF), (HM, D, TQ - TF, TQ)]

    def o_copy(ii, k):
        r0, r1, c0, c1 = o_parts[k]
        q0 = ii * TQ + c0
        if not isinstance(ii, int):
            q0 = pl.multiple_of(q0, LANES)
        return pltpu.make_async_copy(o_ref.at[ii, r0:r1, c0:c1], o_hbm.at[r0:r1, pl.ds(q0, c1 - c0)],
                                     osems.at[0])

    def layernorm(c):
        for t in range(c * TPC, (c + 1) * TPC):
            x = xt_ref[:, t * LANES:(t + 1) * LANES].astype(F32)
            mu = jnp.mean(x, axis=0, keepdims=True)
            xc = x - mu
            var = jnp.mean(xc * xc, axis=0, keepdims=True)
            xnt_sc[t] = (xc * lax.rsqrt(var + EPS)).astype(BF16)

    def xnt_chunk(t0):
        return jnp.concatenate([xnt_sc[t0 + t] for t in range(TPC)], axis=1)

    def proj_k(c):
        kt = jnp.dot(wkt_sc[...], xnt_chunk(c * TPC), preferred_element_type=F32).astype(BF16)
        for gg in range(G):
            kg = kt[gg * GW:(gg + 1) * GW, :].T
            k_sc[gg, c * TC:(c + 1) * TC, :] = kg
            if c * TC < NVR:
                nr = min(TC, NVR - c * TC)
                kf_sc[gg, c * TC:c * TC + nr, :] = kg[:nr, :]

    def proj_v(c):
        vt = jnp.dot(wvt_sc[...], xnt_chunk(zero + c * TPC), preferred_element_type=F32)
        row = lax.broadcasted_iota(jnp.int32, (HP - Dh, TC), 0)
        tail = jnp.where(row == 0, 1.0, 0.0).astype(F32)
        for h in range(H):
            vh = jnp.concatenate([vt[h * Dh:(h + 1) * Dh, :], tail], axis=0)
            vt_sc[h, :, c * TC:(c + 1) * TC] = vh.astype(BF16)

    def q_tile(gg, ii, t):
        qb_sc[0, :, t * LANES:(t + 1) * LANES] = qscale * jnp.dot(
            wqt_sc[gg], xnt_sc[ii * NQT + t], preferred_element_type=F32)

    def kb_index(j, part, d):
        return sum(VUNITS[:j]) * NBC * Dh + (part * Dh + d) * quarter[j]

    def make_kb(src, gg, slot, part, items):
        kf = {}
        for j, d in items:
            nb = quarter[j]
            if nb not in kf:
                r0 = part * (nb * BR)
                if not isinstance(part, int):
                    r0 = pl.multiple_of(r0, nb * BR)
                kf[nb] = src[gg, pl.ds(r0, nb * BR), :].astype(F32)
            kb = jnp.broadcast_to(kf[nb][:, j * Dh + d:j * Dh + d + 1], (nb * BR, LANES))
            kb_sc[pl.ds(slot * KBG + kb_index(j, part, d), nb)] = kb.reshape(nb, BR, LANES)

    def prologue():
        for cp in [wv_copy] + [x_copy(c) for c in range(NC)] + [wqk_copy, wo_copy] + ffn_copies:
            cp.start()
        acc_sc[...] = jnp.zeros(acc_sc.shape, F32)
        wv_copy.wait()
        wvt_sc[...] = wqkv_ref[:, 2 * D:].T
        x_copy(0).wait()
        layernorm(0)
        x_copy(1).wait()
        waited, normed = 2, 1
        for c in range(NC - 1):
            if c + 1 >= waited:
                for cc in range(waited, min(NC, 2 * waited)):
                    x_copy(cc).wait()
                waited = min(NC, 2 * waited)
            if c == NC - 2:
                wqk_copy.wait()
                wo_copy.wait()
            proj_v(c)
            upto = NC if c == NC - 3 else min(c + 2, NC)
            for cc in range(normed, upto):
                layernorm(cc)
            normed = max(normed, upto)
        wqkt = wqkv_ref[:, :2 * D].T
        wkt_sc[...] = wqkt[D:, :]
        for gg in range(G):
            wqt_sc[gg] = wqkt[gg * GW:(gg + 1) * GW, :]
        kb_first = -(-NVR // TC)
        for c in range(NC):
            proj_k(c)
            if c == 1:
                for gg in range(G):
                    wot_sc[gg] = wo_ref[gg * GW:(gg + 1) * GW, :].T
            if kb_first <= c < kb_first + NQ:
                make_kb(k_sc, 0, 0, c - kb_first, kb_items)
        for t in range(NQT):
            q_tile(0, 0, t)
        proj_v(NC - 1)
        for cp in ffn_copies:
            cp.wait()

    def closing(s, pv_acc, rider):
        g, i = s // NQ, s % NQ
        tok0 = pl.multiple_of((i * G + g) * TF, TF)

        def down(rows):
            return xt_ref[rows, pl.ds(tok0, TF)].astype(F32) + lax.dot_general(
                w2t_ref[rows, :], h_sc[...], NT, preferred_element_type=F32)

        lo, hi = slice(0, HM), slice(HM, D)
        pl.when(s > NS - NQ)(lambda: o_copy(i - 1, 2).start())
        r = down(lo)
        outs = [a[:Dh, :] * (1.0 / a[Dh:Dh + 1, :]) for a in pv_acc]
        ot = jnp.concatenate(outs, axis=0).astype(BF16)
        for k, rows in enumerate((lo, hi)):
            at = jnp.dot(wot_sc[g, rows, :], ot, preferred_element_type=F32)
            for t in range(G):
                cols = slice(t * TF, (t + 1) * TF)
                prev = acc_sc[i * G + t, rows, :]
                if k == 0:
                    prev = prev + jnp.where(g == t, r, 0.0)
                a_t = at[:, cols] + prev
                acc_sc[i * G + t, rows, :] = a_t
                if k == 0 or t < G - 1:
                    o_ref[i, rows, cols] = a_t.astype(o_ref.dtype)
            pl.when(g == G - 1)(lambda k=k: o_copy(i, k).start())
        rider(at[KB_ROW:])
        a_t = acc_sc[i * G + g, hi, :] + down(hi)
        acc_sc[i * G + g, hi, :] = a_t
        o_ref[i, hi, TQ - TF:] = a_t.astype(o_ref.dtype)

    def step(s, carry):
        g, i = s // NQ, s % NQ
        sn = (s + 1) % NS
        gn = (g + 1) % G
        zoff = pl.multiple_of(zero * TK, TK)
        kbase = (g % 2) * KBG + zero
        xn_sc[0] = xnt_sc[i * G + g].T
        xn = xn_sc[zero]
        row = lax.broadcasted_iota(jnp.int32, (GW, TQ), 0)

        qm = [None] * HPG
        m_mxu = [None] * HPG
        m_vpu = [None] * HPG
        mx = [None] * HPG
        pv_acc = [None] * HPG
        left = [S] * HPG
        left_mxu = [S - VUNITS[j] * VU for j in range(HPG)]
        chain, fin, toks, cnt = [], [], [], [0]
        vacc, gates = {}, {}

        def fold_max(j, cm, mm, nrows):
            mm[j] = cm if mm[j] is None else jnp.maximum(mm[j], cm)
            left[j] -= nrows
            if mm is m_mxu:
                left_mxu[j] -= nrows
                if left_mxu[j] == 0 and VUNITS[j]:
                    m_sc[j] = m_mxu[j]
            if left[j] == 0:
                full = m_mxu[j] if m_vpu[j] is None else jnp.maximum(m_sc[zero + j], m_vpu[j])
                mx[j] = jnp.max(full, axis=0, keepdims=True)

        def v_step(n, d):
            j, b = vblocks[n]
            accs = vacc.setdefault(n, [None] * NQT)
            ln = j * Dh + d
            kb = kb_sc[kbase + (kb_index(j, b // quarter[j], d) + b % quarter[j])]
            for t in range(NQT):
                pr = kb * qb_sc[zero, ln:ln + 1, t * LANES:(t + 1) * LANES]
                accs[t] = pr if accs[t] is None else accs[t] + pr
            cnt[0] += 1
            if cnt[0] % DS == 0:
                t, v = divmod((cnt[0] // DS * ROT) % (VR * NQT), VR)
                chain.append(accs[t][8 * v:8 * v + 8, :])
                if len(chain) > 1:
                    kb_sc[CH, 0:8, :] = chain.pop(0)
                if fin:
                    kb_sc[CH, 8:16, :] = fin.pop(0)
            if d == Dh - 1:
                st = jnp.concatenate(accs, axis=1)
                s_bufs[j][b * BR:(b + 1) * BR, :] = st
                fold_max(j, jnp.max(st.reshape(VR, 8, TQ), axis=0), m_vpu, BR)
                fin.extend(m_vpu[j][:, t * LANES:(t + 1) * LANES] for t in range(NQT))

        def scores(j, r0, r1):
            if qm[j] is None:
                qm[j] = jnp.where((row >= j * Dh) & (row < (j + 1) * Dh), qb_sc[zero], 0.0).astype(BF16)
            st = jnp.dot(k_sc[g, r0:r1, :], qm[j], preferred_element_type=F32)
            s_bufs[j][r0:r1, :] = st
            fold_max(j, jnp.max(st.reshape((r1 - r0) // 8, 8, TQ), axis=0), m_mxu, r1 - r0)
            toks.append((r1 - r0, st[r1 - r0 - 8:, :]))

        n_early = len(kb_items) * KB_EARLY // 100

        def next_kb(items, tok):
            kf_sc[0, NVR:NVR + BR, :] = tok[0:BR, 0:GW].astype(BF16)
            make_kb(kf_sc, gn + zero, gn % 2, i, items)

        def softmax_pv(j, c):
            if j == 0 and c == 0:
                back, k = 0, len(toks) - 1
                while back < GATE:
                    back += toks[k][0]
                    k -= 1
                s_bufs[0][S:S + 8, :] = toks[k][1]
                s_bufs[0][S:S + 8, :] = m_vpu[vblocks[-1][0]]
            p = jnp.exp2(s_bufs[j][pl.ds(zoff + c * TK, TK), :] - mx[j]).astype(BF16)
            pv = jnp.dot(vt_sc[g * HPG + j, :, c * TK:(c + 1) * TK], p, preferred_element_type=F32)
            pv_acc[j] = pv if c == 0 else pv_acc[j] + pv
            if j == HPG - 1 and c == NCH - 1:
                next_kb(kb_items[:n_early], pv)

        def gate(u, m0, m1):
            gates[(u, m0)] = jnp.dot(xn[m0:m1], w1_ref[:, u * LANES:(u + 1) * LANES],
                                     preferred_element_type=F32)

        def up(u, m0, m1):
            hg = 0.5 * gates.pop((u, m0))
            uu = jnp.dot(xn[m0:m1], w3_ref[:, u * LANES:(u + 1) * LANES], preferred_element_type=F32)
            h_sc[m0:m1, u * LANES:(u + 1) * LANES] = ((hg + hg * jnp.tanh(hg)) * uu).astype(BF16)

        main, riders = [], []

        def add(fn):
            main.append(fn)
            riders.append([])

        add(P(scores, 0, VUNITS[0] * VU, S))
        for u in range(GU0):
            add(P(gate, u, 0, TF))
            add(P(up, u, 0, TF))
        chunks = [(j, c) for j in range(HPG) for c in range(NCH)]
        nxt = 0
        pos = left_mxu[0]
        done_at = [pos]
        nwin = None
        for j in range(1, HPG):
            r0 = VUNITS[j] * VU
            while r0 < S:
                in_win = pos < WIN
                if not in_win and nwin is None:
                    nwin = len(main)
                ready = not in_win and chunks[nxt][0] < j and pos >= done_at[chunks[nxt][0]] + SETTLE
                n = min(PA if ready else TK, S - r0, WIN - pos if in_win else S)
                add(P(scores, j, r0, r0 + n))
                r0 += n
                pos += n
                if ready:
                    riders[-1].append(P(softmax_pv, *chunks[nxt]))
                    nxt += 1
            done_at.append(pos)
        p0 = len(main)
        for t in range(NQT):
            add(P(q_tile, sn // NQ, sn % NQ, t))
        for u in range(GU0, NU):
            for fn in (gate, up):
                for m0 in range(0, TF, PGU):
                    add(P(fn, u, m0, m0 + PGU))
        late = chunks[nxt:]
        for n, jc in enumerate(late):
            riders[p0 + ((n + 1) * (len(main) - p0) - 1) // len(late)].append(P(softmax_pv, *jc))

        vsteps = [(n, d) for n in range(len(vblocks)) for d in range(Dh)]
        for k, fn in enumerate(main):
            if k < nwin:
                for n, d in vsteps[k * len(vsteps) // nwin:(k + 1) * len(vsteps) // nwin]:
                    v_step(n, d)
            fn()
            for rd in riders[k]:
                rd()
        closing(s, pv_acc, P(next_kb, kb_items[n_early:]))
        return carry

    @pl.when(phase == 0)
    def _():
        prologue()
        lax.fori_loop(0, NS, step, 0)
        o_copy(NQ - 1, 2).start()

    @pl.when(phase == 1)
    def _():
        for ii in range(NQ):
            for k in range(len(o_parts)):
                o_copy(ii, k).wait()


@jax.jit
def pallas_parallel_sum__softmax_full_mha__glu_gated_swiglu__prompt_kernel(
    A_x: jax.Array,
    A_wqkv: jax.Array,
    A_wo: jax.Array,
    B_x: jax.Array,
    B_w1: jax.Array,
    B_w3: jax.Array,
    B_w2: jax.Array,
):
    B, S, D = A_x.shape
    F = B_w1.shape[1]
    G = H // HPG
    Dh = D // H
    GW = HPG * Dh
    NQ = S // TQ
    ins = (A_x.reshape(S, D).T, A_wqkv, A_wo, B_w1, B_w3, B_w2.T)
    out = pl.pallas_call(
        functools.partial(_kernel, S=S, D=D, F=F),
        grid=(2,),
        in_specs=[pl.BlockSpec(memory_space=pl.ANY)] * len(ins),
        out_specs=pl.BlockSpec(memory_space=pl.ANY),
        out_shape=jax.ShapeDtypeStruct((D, S), A_x.dtype),
        scratch_shapes=[pltpu.VMEM(a.shape, a.dtype) for a in ins] + [
            pltpu.SemaphoreType.DMA(((S // TC - 1).bit_length() + 4,)),
            pltpu.VMEM((S // LANES, D, LANES), BF16),
            pltpu.VMEM((G, S, GW), BF16),
            pltpu.VMEM((H, HP, S), BF16),
            pltpu.VMEM((D, D), BF16),
            pltpu.VMEM((G, GW, D), BF16),
            pltpu.VMEM((D, D), BF16),
            pltpu.VMEM((G, D, GW), BF16),
            pltpu.VMEM((TQ // G, F), BF16),
            pltpu.VMEM((NQ * G, D, TQ // G), F32),
            pltpu.VMEM((2, TQ // G, D), BF16),
            pltpu.VMEM((2 * sum(VUNITS) * (VU // BR) * Dh + 2, BR, LANES), F32),
            pltpu.VMEM((2, GW, TQ), F32),
            pltpu.VMEM((HPG, 8, TQ), F32),
            pltpu.VMEM((G, max(VUNITS) * VU + 64, GW), BF16),
            pltpu.VMEM((NQ, D, TQ), BF16),
            pltpu.SemaphoreType.DMA((1,)),
        ] + [pltpu.VMEM((S + 8, TQ), F32)] * HPG,
        compiler_params=pltpu.CompilerParams(
            dimension_semantics=("arbitrary",),
            vmem_limit_bytes=110 * 1024 * 1024,
            disable_bounds_checks=True,
        ),
    )(*ins)
    return out.T.reshape(B, S, D)
```
